```python
import os as _os
_os.environ.setdefault("JAX_PLATFORMS", "cpu")
import jax
import jax.numpy as jnp

def _softmax(x, axis=-1):
    return jax.nn.softmax(x, axis=axis)
def _gelu(x):
    return jax.nn.gelu(x, approximate=True)
def _silu(x):
    return jax.nn.silu(x)
def _sigmoid(x):
    return jax.nn.sigmoid(x)
def _layernorm(x, axis=-1, eps=1e-5):
    m = jnp.mean(x, axis=axis, keepdims=True)
    v = jnp.var(x, axis=axis, keepdims=True)
    return (x - m) / jnp.sqrt(v + eps)
def _scatter_add(tgt, idx, src, axis=0):
    return tgt.at[idx].add(src)
def _segment_sum(src, seg, n):
    return jax.ops.segment_sum(src, seg, n)
class _Rng:
    def __init__(self, key):
        self._k = key
    def _next(self):
        self._k, sub = jax.random.split(self._k)
        return sub
    def normal(self, shape):
        return jax.random.normal(self._next(), shape, dtype=jnp.bfloat16)
    def randint(self, lo, hi, shape):
        return jax.random.randint(self._next(), shape, lo, hi, dtype=jnp.int32)
    def uniform(self, shape, lo=0.0, hi=1.0):
        return jax.random.uniform(self._next(), shape, jnp.bfloat16, lo, hi)
    def permutation(self, n):
        return jax.random.permutation(self._next(), n)


kernel_name = 'sequential_preLN__softmax_full_mha__mixer_channel_mlp__prompt'

def setup_inputs():
    _rng = _Rng(jax.random.key(int.from_bytes(__import__("os").urandom(4), "little")))
    _w = (lambda a: (lambda t: t.astype(jnp.bfloat16) if jnp.issubdtype(t.dtype, jnp.floating) else t)(jnp.asarray(a)))
    def _A_setup():
        B, S, D = 1, 2048, 1024
        return {
            "x": _w((lambda *s: _rng.normal(s) * 0.05)(B, S, D)),
            "wqkv": _w((lambda *s: _rng.normal(s) * 0.05)(D, 3 * D)),
            "wo": _w((lambda *s: _rng.normal(s) * 0.05)(D, D)),
        }
    _A_in = _A_setup()

    def _B_setup():
        B, S, D, F = 1, 2048, 1024, 3584
        return {
            "x": _w((lambda *s: _rng.normal(s) * 0.05)(B, S, D)),
            "w1": _w((lambda *s: _rng.normal(s) * 0.8)(D, F) * (D ** -0.5)),
            "b1": _w((lambda *s: _rng.normal(s) * 0.8)(F)),
            "w2": _w((lambda *s: _rng.normal(s) * 0.8)(F, D) * (F ** -0.5)),
            "b2": _w((lambda *s: _rng.normal(s) * 0.05)(D)),
        }
    _B_in = _B_setup()

    return {
        "A_x": _A_in["x"],
        "A_wqkv": _A_in["wqkv"],
        "A_wo": _A_in["wo"],
        "B_x": _B_in["x"],
        "B_w1": _B_in["w1"],
        "B_b1": _B_in["b1"],
        "B_w2": _B_in["w2"],
        "B_b2": _B_in["b2"],
    }

def reference(A_x, A_wqkv, A_wo, B_x, B_w1, B_b1, B_w2, B_b2):
    def _A_ref(x, wqkv, wo):
        B, S, D = x.shape
        H = 32; Dh = D // H
        qkv = (lambda x, *d: x.transpose(*d))((x @ wqkv).reshape(B, S, 3, H, Dh), 2, 0, 3, 1, 4)
        q, k, v = qkv[0], qkv[1], qkv[2]
        scale = Dh ** -0.5
        scores = jnp.einsum("bhqd,bhkd->bhqk", q, k) * scale
        p = _softmax(scores, axis=-1)
        o = jnp.einsum("bhqk,bhkd->bhqd", p, v)
        return (lambda x, *d: x.transpose(*d))(o, 0, 2, 1, 3).reshape(B, S, D) @ wo

    def _B_ref(x, w1, b1, w2, b2):
        y = _layernorm(x, axis=-1)
        h = _gelu(jnp.einsum("bsd,df->bsf", y, w1) + b1)
        return jnp.einsum("bsf,fd->bsd", h, w2) + b2

    x = A_x
    h = x + _A_ref(_layernorm(x, axis=-1), A_wqkv, A_wo)
    h2 = h + _B_ref(_layernorm(h, axis=-1), B_w1, B_b1, B_w2, B_b2)
    return h2
```

```python
import functools
import math

import jax
import jax.numpy as jnp
from jax import lax
from jax.experimental import pallas as pl
from jax.experimental.pallas import tpu as pltpu

f32, bf16, u32 = jnp.float32, jnp.bfloat16, jnp.uint32

S, D, H, DH, F = 2048, 1024, 32, 32, 3584
EPS = 1e-5
QSCALE = (DH ** -0.5) * math.log2(math.e)


def _layernorm(x):
    m = jnp.mean(x, axis=-1, keepdims=True)
    xc = x - m
    v = jnp.mean(xc * xc, axis=-1, keepdims=True)
    return xc * lax.rsqrt(v + EPS)


def _gelu(u):
    c = math.sqrt(2.0 / math.pi)
    z = u * (c + (c * 0.044715) * (u * u))
    hu = 0.5 * u
    return hu + hu * jnp.tanh(z)


def make(name="fused", QB=256, KC=128, skew=4, upi=8, throttle=7, RA=512, SUB=128, FC=512, scopes=False, flags=None):
    NQB = S // QB
    QT = QB // 128
    KT = KC // 128
    NU = NQB * H
    NC = S // KC
    NA = S // RA

    def scope(n):
        if scopes:
            return jax.named_scope(n)
        import contextlib
        return contextlib.nullcontext()

    def kern(x_hbm, wqkv_hbm, wo_hbm, w1_hbm, b1_ref, w2_hbm, b2_ref, out_hbm,
             x_s, wqkv_s, wo_s, w1_s, w2_s, y_s, qT_s, k_s, vT_s, w_a, w_b, s_a, s_b, oT_s,
             h_s, y2_s, u_s, out_s, sem_x, sem_w, sem_o):
        def x_copy(i):
            return pltpu.make_async_copy(x_hbm.at[0, pl.ds(i * RA, RA), :], x_s.at[pl.ds(i * RA, RA), :], sem_x.at[i])

        def wqkv_copy(j):
            return pltpu.make_async_copy(wqkv_hbm.at[:, pl.ds(j * D, D)], wqkv_s.at[j], sem_w.at[j])

        wo_copy = pltpu.make_async_copy(wo_hbm, wo_s, sem_w.at[3])
        w1_copy = pltpu.make_async_copy(w1_hbm, w1_s, sem_w.at[4])
        w2_copy = pltpu.make_async_copy(w2_hbm, w2_s, sem_w.at[5])

        def out_copy(qb, slot):
            return pltpu.make_async_copy(out_s.at[slot], out_hbm.at[0, pl.ds(pl.multiple_of(qb * QB, QB), QB), :], sem_o.at[slot])

        x_copy(0).start()
        for j in range(3):
            wqkv_copy(j).start()
        for i in range(1, NA):
            x_copy(i).start()
        wo_copy.start()
        w1_copy.start()
        w2_copy.start()

        with scope("wait0"):
            for j in range(3):
                wqkv_copy(j).wait()

        def phase_a(i, c):
            x_copy(i).wait()
            r0 = pl.multiple_of(i * RA, RA)
            for sb in range(RA // SUB):
                xs = x_s[pl.ds(r0 + sb * SUB, SUB), :].astype(f32)
                y_s[sb * SUB:(sb + 1) * SUB, :] = _layernorm(xs).astype(bf16)
            y = y_s[...]
            for half in range(2):
                cs = slice(half * 512, (half + 1) * 512)
                kk = jnp.dot(y, wqkv_s[1, :, cs], preferred_element_type=f32).astype(bf16)
                for g in range(4):
                    k_s[half * 4 + g, pl.ds(pl.multiple_of(i * (RA // 2), RA // 2), RA // 2), :] = pltpu.bitcast(kk[:, g * 128:(g + 1) * 128], u32)
            for half in range(2):
                cs = slice(half * 512, (half + 1) * 512)
                q = (jnp.dot(y, wqkv_s[0, :, cs], preferred_element_type=f32) * QSCALE).astype(bf16)
                qt = q.T
                for t in range(RA // 128):
                    qT_s[i * (RA // 128) + t, cs, :] = qt[:, t * 128:(t + 1) * 128]
            for half in range(2):
                cs = slice(half * 512, (half + 1) * 512)
                v = jnp.dot(y, wqkv_s[2, :, cs], preferred_element_type=f32).astype(bf16)
                vt = v.T
                for t in range(RA // 128):
                    vT_s[i * (RA // 128) + t, cs, :] = vt[:, t * 128:(t + 1) * 128]
            return c

        with scope("phaseA"):
            lax.fori_loop(0, NA, phase_a, 0)

        ws = (w_a, w_b)
        ss = (s_a, s_b)

        def prep_w(u, w_s):
            qb = u // H
            h = u % H
            g = h // 4
            j = h % 4
            row = lax.broadcasted_iota(jnp.int32, (128, 128), 0)
            keep = (row >= j * DH) & (row < j * DH + DH)
            for t in range(QT):
                q = qT_s[qb * QT + t, pl.ds(pl.multiple_of(g * 128, 128), 128), :]
                w = jnp.where(keep, q.astype(f32), 0.0).astype(bf16)
                w_s[t] = pltpu.bitcast(w, u32)

        def qk_chunk(u, c, w_s, s_s, m):
            g = (u % H) // 4
            w = jnp.concatenate([pltpu.bitcast(w_s[t], bf16) for t in range(QT)], axis=1)
            k = pltpu.bitcast(k_s[g, c * KC // 2:(c + 1) * KC // 2, :], bf16)
            s = jnp.dot(k, w, preferred_element_type=f32)
            s_s[c * KC:(c + 1) * KC, :] = s
            for r in range(KC // 8):
                xr = s[r * 8:(r + 1) * 8]
                m = xr if m is None else jnp.maximum(m, xr)
            return m

        def pv_chunk(u, c, s_s, mb, l, acc):
            h = u % H
            ps = []
            for r in range(KC // 16):
                p0 = jnp.exp2(s_s[c * KC + r * 16: c * KC + r * 16 + 8, :] - mb)
                p1 = jnp.exp2(s_s[c * KC + r * 16 + 8: c * KC + r * 16 + 16, :] - mb)
                t = p0 + p1
                l = t if l is None else l + t
                ps += [p0, p1]
            pb = jnp.concatenate(ps, axis=0).astype(bf16)
            v = jnp.concatenate([vT_s[c * KT + t, pl.ds(pl.multiple_of(h * DH, DH), DH), :] for t in range(KT)], axis=1)
            a = jnp.dot(v, pb, preferred_element_type=f32)
            acc = a if acc is None else acc + a
            return l, acc

        def fin(u, l, acc):
            h = u % H
            lt = jnp.sum(l, axis=0, keepdims=True)
            o = (acc * (1.0 / lt)).astype(bf16)
            for t in range(QT):
                oT_s[t, pl.ds(pl.multiple_of(h * DH, DH), DH), :] = o[:, t * 128:(t + 1) * 128]

        def bmax(m):
            return jnp.broadcast_to(jnp.max(m, axis=0, keepdims=True), (8, QB))

        def clampu(u):
            return jnp.minimum(u, NU - 1)

        def half_step(u, par, mb, m, hist):
            l = None
            acc = None
            mb_next = None
            for c in range(NC):
                cq = c + skew
                if cq < NC:
                    m = qk_chunk(clampu(u + 1), cq, ws[1 - par], ss[1 - par], m)
                    if cq == NC - 1:
                        mb_next = bmax(m)
                        m = None
                else:
                    m = qk_chunk(clampu(u + 2), cq - NC, ws[par], ss[par], m)
                if c == 4:
                    prep_w(clampu(u + 2), ws[par])
                hist.append(m if m is not None else mb_next)
                mbc = mb
                if throttle and len(hist) >= throttle:
                    mbc = jnp.maximum(mb, jnp.minimum(mb, hist[-throttle]))
                l, acc = pv_chunk(u, c, ss[par], mbc, l, acc)
            fin(u, l, acc)
            return mb_next, m

        with scope("attn_prologue"):
            prep_w(0, w_a)
            prep_w(1, w_b)
            m = None
            for c in range(NC):
                m = qk_chunk(0, c, w_a, s_a, m)
            mb = bmax(m)
            m = None
            for c in range(skew):
                m = qk_chunk(1, c, w_b, s_b, m)

        with scope("wait1"):
            wo_copy.wait()
            w1_copy.wait()
            w2_copy.wait()

        def phase_c(qb):
            slot = qb % 2
            b1 = b1_ref[...].astype(f32).reshape(1, F)
            b2 = b2_ref[...].astype(f32).reshape(1, D)
            r0 = pl.multiple_of(qb * QB, QB)
            for t in range(QT):
                rs = slice(t * 128, (t + 1) * 128)
                a = lax.dot_general(oT_s[t], wo_s[...], (((0,), (0,)), ((), ())), preferred_element_type=f32)
                hh = x_s[pl.ds(r0 + t * 128, 128), :].astype(f32) + a
                h_s[rs, :] = hh
                y2_s[rs, :] = _layernorm(hh).astype(bf16)
            for t in range(QT):
                rs = slice(t * 128, (t + 1) * 128)
                y2 = y2_s[rs, :]
                for j in range(F // FC):
                    cs = slice(j * FC, (j + 1) * FC)
                    u = jnp.dot(y2, w1_s[:, cs], preferred_element_type=f32) + b1[:, cs]
                    u_s[rs, cs] = _gelu(u).astype(bf16)

            @pl.when(qb >= 2)
            def _():
                out_copy(qb - 2, slot).wait()

            for t in range(QT):
                rs = slice(t * 128, (t + 1) * 128)
                o = jnp.dot(u_s[rs, :], w2_s[...], preferred_element_type=f32)
                out_s[slot, rs, :] = (h_s[rs, :] + (o + b2)).astype(bf16)
            out_copy(qb, slot).start()

        def qblock(qb, carry):
            def step(i, carry):
                mb, m = carry
                hist = []
                for j in range(upi):
                    mb, m = half_step(qb * H + upi * i + j, j % 2, mb, m, hist)
                return mb, m

            with scope("attn"):
                carry = lax.fori_loop(0, H // upi, step, carry)
            with scope("phaseC"):
                phase_c(qb)
            return carry

        lax.fori_loop(0, NQB, qblock, (mb, m))
        with scope("wait2"):
            out_copy(NQB - 2, 0).wait()
            out_copy(NQB - 1, 1).wait()

    def run(A_x, A_wqkv, A_wo, B_x, B_w1, B_b1, B_w2, B_b2):
        del B_x
        anyspec = pl.BlockSpec(memory_space=pl.ANY)
        vmem = pl.BlockSpec(memory_space=pltpu.VMEM)
        return pl.pallas_call(
            kern,
            out_shape=jax.ShapeDtypeStruct((1, S, D), bf16),
            in_specs=[anyspec, anyspec, anyspec, anyspec, vmem, anyspec, vmem],
            out_specs=anyspec,
            scratch_shapes=[
                pltpu.VMEM((S, D), bf16),
                pltpu.VMEM((3, D, D), bf16),
                pltpu.VMEM((D, D), bf16),
                pltpu.VMEM((D, F), bf16),
                pltpu.VMEM((F, D), bf16),
                pltpu.VMEM((RA, D), bf16),
                pltpu.VMEM((16, D, 128), bf16),
                pltpu.VMEM((8, S // 2, 128), u32),
                pltpu.VMEM((16, D, 128), bf16),
                pltpu.VMEM((QT, 64, 128), u32),
                pltpu.VMEM((QT, 64, 128), u32),
                pltpu.VMEM((S, QB), f32),
                pltpu.VMEM((S, QB), f32),
                pltpu.VMEM((QT, D, 128), bf16),
                pltpu.VMEM((QB, D), f32),
                pltpu.VMEM((QB, D), bf16),
                pltpu.VMEM((QB, F), bf16),
                pltpu.VMEM((2, QB, D), bf16),
                pltpu.SemaphoreType.DMA((NA,)),
                pltpu.SemaphoreType.DMA((6,)),
                pltpu.SemaphoreType.DMA((2,)),
            ],
            compiler_params=pltpu.CompilerParams(vmem_limit_bytes=100 << 20, flags=flags),
            name=name,
        )(A_x, A_wqkv, A_wo, B_w1, B_b1, B_w2, B_b2)

    return run


@jax.jit
def pallas_sequential_preLN__softmax_full_mha__mixer_channel_mlp__prompt_kernel(
    A_x, A_wqkv, A_wo, B_x, B_w1, B_b1, B_w2, B_b2
):
    return make()(A_x, A_wqkv, A_wo, B_x, B_w1, B_b1, B_w2, B_b2)
```

```python
import contextlib
import math

import jax
import jax.numpy as jnp
from jax import lax
from jax.experimental import pallas as pl
from jax.experimental.pallas import tpu as pltpu

f32, bf16, u32 = jnp.float32, jnp.bfloat16, jnp.uint32

S, D, H, DH, F = 2048, 1024, 32, 32, 3584
D2, D4, F4 = D // 2, D // 4, F // 4
QB = 256
NQB = S // QB
KC = 128
NC = S // KC
NU = NQB * H
EPS = 1e-5
QSCALE = (DH ** -0.5) * math.log2(math.e)
QUADS = ((0, 0), (0, 1), (1, 0), (1, 1))


def _layernorm(x):
    m = jnp.mean(x, axis=-1, keepdims=True)
    xc = x - m
    v = jnp.mean(xc * xc, axis=-1, keepdims=True)
    return xc * lax.rsqrt(v + EPS)


def _gelu(u):
    c = math.sqrt(2.0 / math.pi)
    z = u * (c + (c * 0.044715) * (u * u))
    hu = 0.5 * u
    return hu + hu * jnp.tanh(z)


def _dot(a, b):
    return jnp.dot(a, b, preferred_element_type=f32)


def _pack(a):
    return pltpu.bitcast(a.astype(bf16), u32)


def _unpack(w):
    return pltpu.bitcast(w, bf16)


def _lhs(ref, p, rows=slice(None)):
    return jnp.concatenate([_unpack(ref[p, t, rows, :]) for t in range(ref.shape[1])], axis=1)


def _after(x, t):
    t = jnp.tile(t, (x.shape[0] // t.shape[0], x.shape[1] // t.shape[1]))
    return jnp.maximum(x, jnp.minimum(x, t))


def _lhs_factors(a11, a12, a21, a22):
    return [a11 + a22, a21 + a22, a11, a22, a11 + a12, a21 - a11, a12 - a22]


def _rhs_factors(b11, b12, b21, b22):
    return [b11 + b22, b11, b12 - b22, b21 - b11, b22, b11 + b12, b21 + b22]


_RHS_TERMS = ((0, 3, 1), (0, None, 0), (1, 3, -1), (2, 0, -1), (3, None, 0), (0, 1, 1), (2, 3, 1))


def _lhs_factors2(a):
    outer = [_lhs_factors(a[r][c], a[r][2 + c], a[2 + r][c], a[2 + r][2 + c]) for r, c in QUADS]
    return [v for p in range(7) for v in _lhs_factors(*(outer[q][p] for q in range(4)))]


class _Quad:
    def __init__(self, v):
        self.v = v

    def __add__(self, o):
        return _Quad([a + b for a, b in zip(self.v, o.v)])

    def __sub__(self, o):
        return _Quad([a - b for a, b in zip(self.v, o.v)])


def _combine(prod, first=()):
    done = {p: prod(p) for p in first}

    def m(p):
        return done[p] if p in done else prod(p)

    m0 = m(0)
    c11 = m0 + m(6)
    m3 = m(3)
    c11 = c11 + m3
    m4 = m(4)
    c11 = c11 - m4
    m2 = m(2)
    c12 = m2 + m4
    c22 = m0 + m2
    m1 = m(1)
    c21 = m1 + m3
    c22 = (c22 - m1) + m(5)
    return c11, c12, c21, c22


def _combine2(prod, first=()):
    out = _combine(lambda p: _Quad(_combine(lambda q: prod(7 * p + q))), first)
    c = [[None] * 4 for _ in range(4)]
    for po, (ro, co) in enumerate(QUADS):
        for q, (r, cc) in enumerate(QUADS):
            c[2 * ro + r][2 * co + cc] = out[po].v[q]
    return c


def make(name="fused", skew=4, upi=16, throttle=6, qv_unroll=2, scopes=False, fine=None, flags=None, sched=None,
         vmem_mb=120, cut=3):
    if sched is None:
        sched = {'start': ['x0', 'k0', 'k1'], 'x0': ['k2', 'x1'], 'k0': ['k3'], 'k1': ['x2'], 'x1': ['q', 'v'], 'x2': ['x5']}
    xb = (0, 256, 512, 1280, 2048)
    NIT = NU // upi

    def scope(n):
        return jax.named_scope(n) if scopes else contextlib.nullcontext()

    def kern(x_hbm, wqkv_hbm, wo_hbm, w1_hbm, b1_ref, w2_hbm, b2_ref, out_hbm,
             x_s, wo_s, w1_s, w2_s, qT_s, k_s, vT_s, sem_x, sem_k, sem_w, sem_o):
        wo_copy = pltpu.make_async_copy(wo_hbm, wo_s, sem_w.at[2])
        w1_copy = pltpu.make_async_copy(w1_hbm, w1_s, sem_w.at[3])
        w2_copy = pltpu.make_async_copy(w2_hbm, w2_s, sem_w.at[4])

        def projections(wk_s, wq_s, wv_s, wkb_s, wqb_s, wvb_s, y_s):
            cp = {}
            for i in range(len(xb) - 1):
                rows = pl.ds(xb[i], xb[i + 1] - xb[i])
                cp[f"x{xb[i] // QB}"] = pltpu.make_async_copy(x_hbm.at[0, rows, :], x_s.at[rows, :], sem_x.at[i])
            for j in range(4):
                cp[f"k{j}"] = pltpu.make_async_copy(wqkv_hbm.at[:, pl.ds(D + j * 256, 256)], wk_s.at[j], sem_k.at[j])
            cp["q"] = pltpu.make_async_copy(wqkv_hbm.at[:, pl.ds(0, D)], wq_s, sem_w.at[0])
            cp["v"] = pltpu.make_async_copy(wqkv_hbm.at[:, pl.ds(2 * D, D)], wv_s, sem_w.at[1])

            def wait(tag):
                with scope("w" + tag):
                    cp[tag].wait()
                for t in sched.get(tag, ()):
                    cp[t].start()

            for t in sched["start"]:
                cp[t].start()

            def ln_piece(i, p, dep=None):
                r = p * 8
                x0 = x_s[i * QB + r:i * QB + r + 8, :].astype(f32)
                x1 = x_s[i * QB + 128 + r:i * QB + 128 + r + 8, :].astype(f32)
                if dep is not None:
                    x0 = jnp.concatenate([_after(x0[:, :128], dep), x0[:, 128:]], axis=1)
                    x1 = jnp.concatenate([_after(x1[:, :128], dep), x1[:, 128:]], axis=1)
                y0, y1 = _layernorm(x0), _layernorm(x1)
                for n, a in enumerate(_lhs_factors(y0[:, :D2], y0[:, D2:], y1[:, :D2], y1[:, D2:])):
                    y_s[n, i * 128 + r:i * 128 + r + 8, :] = a.astype(bf16)

            def prep(src, dst, j, r, dep=None):
                top, bot = src[r:r + 16, :].astype(f32), src[D2 + r:D2 + r + 16, :].astype(f32)
                b11, b12, b21, b22 = top[:, :128], top[:, 128:], bot[:, :128], bot[:, 128:]
                if dep is not None:
                    b11, b22 = _after(b11, dep), _after(b22, dep)
                for n, b in enumerate(_rhs_factors(b11, b12, b21, b22)):
                    if n not in (1, 4):
                        dst[j, n, r:r + 16, :] = b.astype(bf16)

            last = [None]

            def products(src, dst, j, rows, before=None):
                def prod(p):
                    if before is not None:
                        before()
                    if p == 1:
                        b = src[:D2, :128]
                    elif p == 4:
                        b = src[D2:, 128:]
                    else:
                        b = dst[j, p]
                    last[0] = _dot(y_s[p, rows, :], b)
                    return last[0]
                return prod

            with scope("phaseA_k"):
                wait("x0")
                for p in range(16):
                    ln_piece(0, p)
                qv_jobs = [(w.at[:, pl.ds(j * 256, 256)], wb, j, r) for w, wb in ((wq_s, wqb_s), (wv_s, wvb_s))
                           for j in range(4) for r in range(0, D2, 16)]
                for i in range(NQB):
                    count = [0]
                    ln_from = {0: 22, 1: 15}.get(i, 0)

                    def side_work():
                        d = count[0]
                        count[0] += 1
                        if i + 1 < NQB and d >= ln_from:
                            n = 26 - ln_from
                            for p in range((d - ln_from) * 16 // n, min(16, (d - ln_from + 1) * 16 // n)):
                                ln_piece(i + 1, p, last[0][(p % 4) * 32:(p % 4) * 32 + 8])
                        if i >= 4:
                            n0 = (i - 4) * 28 + d
                            for p in range(n0 * len(qv_jobs) // 112, (n0 + 1) * len(qv_jobs) // 112):
                                prep(*qv_jobs[p], last[0][32 + 64 * (p % 2):32 + 64 * (p % 2) + 8])

                    if i == 4:
                        wait("x5")
                        wait("q")
                        wait("v")
                    for j in range(4):
                        if i == 0:
                            wait(f"k{j}")
                            if j == 3:
                                wait("x1")
                            for r in range(0, D2, 16):
                                prep(wk_s.at[j], wkb_s, j, r)
                        if i == 1 and j == 2:
                            wait("x2")
                        c = _combine(products(wk_s.at[j], wkb_s, j, slice(i * 128, (i + 1) * 128), side_work),
                                     first=(1, 4) if i == 0 else ())
                        for (t, g), val in zip(QUADS, c):
                            k_s[2 * j + g, i * 128 + t * 64:i * 128 + (t + 1) * 64, :] = _pack(val)

            def qv_step(it, carry):
                @pl.when(it == 1)
                def _():
                    wo_copy.start()
                    w1_copy.start()
                    w2_copy.start()

                for sub in range(qv_unroll):
                    i = it * qv_unroll + sub
                    rows = pl.ds(pl.multiple_of(i * 128, 128), 128)
                    for w, wb, dst, scale in ((wq_s, wqb_s, qT_s, QSCALE), (wv_s, wvb_s, vT_s, None)):
                        for j in range(4):
                            c = _combine(products(w.at[:, pl.ds(j * 256, 256)], wb, j, rows))
                            for (t, g), val in zip(QUADS, c):
                                if scale is not None:
                                    val = val * scale
                                dst[2 * i + t, (2 * j + g) * 128:(2 * j + g + 1) * 128, :] = val.astype(bf16).T
                return carry

            with scope("phaseA_qv"):
                lax.fori_loop(0, NQB // qv_unroll, qv_step, 0)

        pl.run_scoped(
            projections,
            pltpu.VMEM((4, D, 256), bf16), pltpu.VMEM((D, D), bf16), pltpu.VMEM((D, D), bf16),
            pltpu.VMEM((4, 7, D2, 128), bf16), pltpu.VMEM((4, 7, D2, 128), bf16),
            pltpu.VMEM((4, 7, D2, 128), bf16), pltpu.VMEM((7, S // 2, D2), bf16))

        def rest(wob_s, w1b_s, w2b_s, w_a, w_b, s_a, s_b, oT_s, oa_s, h_s, y0_s, ya_s, ua_s, out_s):
            ws = (w_a, w_b)
            ss = (s_a, s_b)

            def prep_w(u, w_s):
                qb = u // H
                h = u % H
                g = h // 4
                j = h % 4
                row = lax.broadcasted_iota(jnp.int32, (128, 128), 0)
                keep = (row >= j * DH) & (row < j * DH + DH)
                for t in range(2):
                    q = qT_s[qb * 2 + t, pl.ds(pl.multiple_of(g * 128, 128), 128), :]
                    w_s[t] = _pack(jnp.where(keep, q.astype(f32), 0.0))

            def qk_chunk(u, c, w_s, s_s, m):
                g = (u % H) // 4
                w = jnp.concatenate([_unpack(w_s[t]) for t in range(2)], axis=1)
                s = _dot(_unpack(k_s[g, c * KC // 2:(c + 1) * KC // 2, :]), w)
                s_s[c * KC:(c + 1) * KC, :] = s
                for r in range(KC // 8):
                    xr = s[r * 8:(r + 1) * 8]
                    m = xr if m is None else jnp.maximum(m, xr)
                return m

            def pv_chunk(u, c, s_s, mb, l, acc):
                h = u % H
                ps = []
                for r in range(KC // 16):
                    p0 = jnp.exp2(s_s[c * KC + r * 16: c * KC + r * 16 + 8, :] - mb)
                    p1 = jnp.exp2(s_s[c * KC + r * 16 + 8: c * KC + r * 16 + 16, :] - mb)
                    t = p0 + p1
                    l = t if l is None else l + t
                    ps += [p0, p1]
                pb = jnp.concatenate(ps, axis=0).astype(bf16)
                a = _dot(vT_s[c, pl.ds(pl.multiple_of(h * DH, DH), DH), :], pb)
                acc = a if acc is None else acc + a
                return l, acc

            def fin(u, l, acc):
                qb = u // H
                h = u % H
                o = acc * (1.0 / jnp.sum(l, axis=0, keepdims=True))
                for t in range(2):
                    oT_s[qb * 2 + t, pl.ds(pl.multiple_of(h * DH, DH), DH), :] = o[:, t * 128:(t + 1) * 128]

            def bmax(m):
                return jnp.broadcast_to(jnp.max(m, axis=0, keepdims=True), (8, QB))

            def clampu(u):
                return jnp.minimum(u, NU - 1)

            def weight_jobs(it):
                jobs = []

                def two_level(src, dst, kq, nq, r0, n, p):
                    def blk(r, c):
                        return src[pl.ds(r * kq + r0, 16), c * nq + n * 128:c * nq + (n + 1) * 128].astype(f32)

                    outer = []

                    def first(dep):
                        qa, qb, sign = _RHS_TERMS[p]
                        for r, c in QUADS:
                            v = blk(2 * QUADS[qa][0] + r, 2 * QUADS[qa][1] + c)
                            if r == c:
                                v = _after(v, dep)
                            if sign:
                                v2 = blk(2 * QUADS[qb][0] + r, 2 * QUADS[qb][1] + c)
                                v = v + v2 if sign > 0 else v - v2
                            outer.append(v)
                        emit(range(cut), None)

                    def emit(qs, dep):
                        o = list(outer)
                        if dep is not None:
                            o[0], o[3] = _after(o[0], dep), _after(o[3], dep)
                        vals = _rhs_factors(*o)
                        for q in qs:
                            dst[7 * p + q, n, pl.ds(pl.multiple_of(r0 // 2, 8), 8), :] = _pack(vals[q])

                    jobs.append(first)
                    if cut < 7:
                        jobs.append(lambda dep: emit(range(cut, 7), dep))

                for a in range(D4 // 16 // NIT):
                    r0 = pl.multiple_of((it * (D4 // 16 // NIT) + a) * 16, 16)
                    for n in range(F4 // 128):
                        for p in range(7):
                            two_level(w1_s, w1b_s, D4, F4, r0, n, p)
                ng = -(-(F4 // 16) // NIT)
                for a in range(ng):
                    r0 = pl.multiple_of(jnp.minimum(it * ng + a, F4 // 16 - 1) * 16, 16)
                    for n in range(D4 // 128):
                        for p in range(7):
                            two_level(w2_s, w2b_s, F4, D4, r0, n, p)
                for a in range(D2 // 16 // NIT):
                    r0 = pl.multiple_of((it * (D2 // 16 // NIT) + a) * 16, 16)
                    for j in range(4):
                        def run(dep, j=j, r0=r0):
                            top = _after(wo_s[pl.ds(r0, 16), j * 256:(j + 1) * 256].astype(f32), dep)
                            bot = wo_s[pl.ds(D2 + r0, 16), j * 256:(j + 1) * 256].astype(f32)
                            for n, b in enumerate(_rhs_factors(top[:, :128], top[:, 128:], bot[:, :128], bot[:, 128:])):
                                wob_s[j, n, pl.ds(pl.multiple_of(r0 // 2, 8), 8), :] = _pack(b)
                        jobs.append(run)
                return jobs

            def unit(it, j, mb, m, hist, jobs):
                u = upi * it + j
                par = j % 2
                l = None
                acc = None
                mb_next = None
                for c in range(NC):
                    cq = c + skew
                    if cq < NC:
                        m = qk_chunk(clampu(u + 1), cq, ws[1 - par], ss[1 - par], m)
                        if cq == NC - 1:
                            mb_next = bmax(m)
                            m = None
                    else:
                        m = qk_chunk(clampu(u + 2), cq - NC, ws[par], ss[par], m)
                    if c == 4:
                        prep_w(clampu(u + 2), ws[par])
                    hist.append(m if m is not None else mb_next)
                    n0, n1 = j * NC + c, upi * NC
                    for p in range(n0 * len(jobs) // n1, (n0 + 1) * len(jobs) // n1):
                        jobs[p](hist[-1][:, :128])
                    mbc = _after(mb, hist[-throttle]) if len(hist) >= throttle else mb
                    l, acc = pv_chunk(u, c, ss[par], mbc, l, acc)
                fin(u, l, acc)
                return mb_next, m

            with scope("attn_prologue"):
                wo_copy.wait()
                w1_copy.wait()
                w2_copy.wait()
                prep_w(0, w_a)
                prep_w(1, w_b)
                m = None
                for c in range(NC):
                    m = qk_chunk(0, c, w_a, s_a, m)
                mb = bmax(m)
                m = None
                for c in range(skew):
                    m = qk_chunk(1, c, w_b, s_b, m)

            def attn_step(it, carry):
                mb, m = carry
                hist = []
                jobs = weight_jobs(it)
                for j in range(upi):
                    mb, m = unit(it, j, mb, m, hist, jobs)
                return mb, m

            with scope("attn"):
                lax.fori_loop(0, NIT, attn_step, (mb, m))

            def out_copy(qb, slot):
                return pltpu.make_async_copy(
                    out_s.at[slot], out_hbm.at[0, pl.ds(pl.multiple_of(qb * QB, QB), QB), :], sem_o.at[slot])

            def prep_o(qb, t, g, dep=None):
                lo = oT_s[2 * qb + t, g * 128:(g + 1) * 128, :]
                hi = oT_s[2 * qb + t, D2 + g * 128:D2 + (g + 1) * 128, :]
                if dep is not None:
                    lo, hi = _after(lo, dep), _after(hi, dep)
                lo, hi = lo.T, hi.T
                for n, a in enumerate(_lhs_factors(lo[:64], hi[:64], lo[64:], hi[64:])):
                    oa_s[7 * t + n, g] = _pack(a)

            def mlp_step(qb, carry):
                slot = qb % 2

                @pl.when(qb >= 2)
                def _():
                    out_copy(qb - 2, slot).wait()

                b1 = b1_ref[...].astype(f32).reshape(1, F)
                b2 = b2_ref[...].astype(f32).reshape(1, D)
                r0 = pl.multiple_of(qb * QB, QB)

                def grid(ys, t):
                    return [[y[:, cq * D4 + t * 128:cq * D4 + (t + 1) * 128] for cq in range(4)] for y in ys]

                for t in range(2):
                    for j in range(4):
                        c = _combine(lambda p: _dot(_lhs(oa_s, 7 * t + p), _unpack(wob_s[j, p])))
                        for (r, g), val in zip(QUADS, c):
                            cs = slice((2 * j + g) * 128, (2 * j + g + 1) * 128)
                            ro = t * 128 + r * 64
                            h_s[ro:ro + 64, cs] = x_s[pl.ds(r0 + ro, 64), cs].astype(f32) + val
                    for r in range(0, 64, 16):
                        ys = [_layernorm(h_s[t * 128 + q * 64 + r:t * 128 + q * 64 + r + 16, :]) for q in range(2)]
                        if t == 0:
                            for q in range(2):
                                y0_s[q * 64 + r:q * 64 + r + 16, :] = ys[q]
                            for kt in range(2):
                                a = grid(ys, kt)
                                top = [(a[q][c], a[q][c] + a[q][2 + c]) for q, c in QUADS]
                                for p, sel in ((2, 0), (4, 1)):
                                    for n, v in enumerate(_lhs_factors(*(o[sel] for o in top))):
                                        ya_s[7 * p + n, kt, r // 2:r // 2 + 8, :] = _pack(v)
                        else:
                            ys = [y0_s[q * 64 + r:q * 64 + r + 16, :] for q in range(2)] + ys
                            for kt in range(2):
                                for n, v in enumerate(_lhs_factors2(grid(ys, kt))):
                                    if n // 7 not in (2, 4):
                                        ya_s[n, kt, r // 2:r // 2 + 8, :] = _pack(v)

                for n in range(F4 // 128):
                    c = _combine2(lambda p: _dot(_lhs(ya_s, p), _unpack(w1b_s[p, n])), first=(2, 4) if n == 0 else ())
                    for r in range(0, 64, 16):
                        u = [[_gelu(c[t][cq][r:r + 16] + b1[:, cq * F4 + n * 128:cq * F4 + (n + 1) * 128])
                              for cq in range(4)] for t in range(4)]
                        for p, a in enumerate(_lhs_factors2(u)):
                            ua_s[p, n, r // 2:r // 2 + 8, :] = _pack(a)

                nxt = jnp.minimum(qb + 1, NQB - 1)
                for n in range(D4 // 128):
                    count = [0]

                    def prod(p):
                        val = _dot(_lhs(ua_s, p), _unpack(w2b_s[p, n]))
                        d = count[0]
                        count[0] += 1
                        if d % 12 == 2:
                            prep_o(nxt, n, d // 12, val[:8])
                        return val

                    c = _combine2(prod)
                    for t in range(4):
                        for cq in range(4):
                            rs, cs = slice(t * 64, (t + 1) * 64), slice(cq * D4 + n * 128, cq * D4 + (n + 1) * 128)
                            out_s[slot, rs, cs] = (h_s[rs, cs] + (c[t][cq] + b2[:, cs])).astype(bf16)
                out_copy(qb, slot).start()
                return carry

            with scope("phaseC"):
                for t in range(2):
                    for g in range(4):
                        prep_o(0, t, g)
                lax.fori_loop(0, NQB, mlp_step, 0)
            with scope("wait2"):
                out_copy(NQB - 2, 0).wait()
                out_copy(NQB - 1, 1).wait()

        pl.run_scoped(
            rest,
            pltpu.VMEM((4, 7, D2 // 2, 128), u32),
            pltpu.VMEM((49, F4 // 128, D4 // 2, 128), u32),
            pltpu.VMEM((49, D4 // 128, F4 // 2, 128), u32),
            pltpu.VMEM((2, 64, 128), u32),
            pltpu.VMEM((2, 64, 128), u32),
            pltpu.VMEM((S, QB), f32),
            pltpu.VMEM((S, QB), f32),
            pltpu.VMEM((S // 128, D, 128), f32),
            pltpu.VMEM((14, 4, 32, 128), u32),
            pltpu.VMEM((QB, D), f32),
            pltpu.VMEM((128, D), f32),
            pltpu.VMEM((49, D4 // 128, 32, 128), u32),
            pltpu.VMEM((49, F4 // 128, 32, 128), u32),
            pltpu.VMEM((2, QB, D), bf16))

    def run(A_x, A_wqkv, A_wo, B_x, B_w1, B_b1, B_w2, B_b2):
        del B_x
        anyspec = pl.BlockSpec(memory_space=pl.ANY)
        vmem = pl.BlockSpec(memory_space=pltpu.VMEM)
        return pl.pallas_call(
            kern,
            out_shape=jax.ShapeDtypeStruct((1, S, D), bf16),
            in_specs=[anyspec, anyspec, anyspec, anyspec, vmem, anyspec, vmem],
            out_specs=anyspec,
            scratch_shapes=[
                pltpu.VMEM((S, D), bf16),
                pltpu.VMEM((D, D), bf16),
                pltpu.VMEM((D, F), bf16),
                pltpu.VMEM((F, D), bf16),
                pltpu.VMEM((S // 128, D, 128), bf16),
                pltpu.VMEM((8, S // 2, 128), u32),
                pltpu.VMEM((S // 128, D, 128), bf16),
                pltpu.SemaphoreType.DMA((len(xb) - 1,)),
                pltpu.SemaphoreType.DMA((4,)),
                pltpu.SemaphoreType.DMA((5,)),
                pltpu.SemaphoreType.DMA((2,)),
            ],
            compiler_params=pltpu.CompilerParams(vmem_limit_bytes=vmem_mb << 20, flags=flags),
            name=name,
        )(A_x, A_wqkv, A_wo, B_w1, B_b1, B_w2, B_b2)

    return run


@jax.jit
def pallas_sequential_preLN__softmax_full_mha__mixer_channel_mlp__prompt_kernel(
    A_x, A_wqkv, A_wo, B_x, B_w1, B_b1, B_w2, B_b2
):
    return make()(A_x, A_wqkv, A_wo, B_x, B_w1, B_b1, B_w2, B_b2)
```

```python
import math

import jax
import jax.numpy as jnp
from jax import lax
from jax.experimental import pallas as pl
from jax.experimental.pallas import tpu as pltpu

f32, bf16, u32 = jnp.float32, jnp.bfloat16, jnp.uint32

S, D, H, DH, F = 2048, 1024, 32, 32, 3584
D2, D4, F4 = D // 2, D // 4, F // 4
QB = 256
NQB = S // QB
KC = 128
NC = S // KC
NU = NQB * H
UNROLL = 16
NIT = NU // UNROLL
SKEW = 4
LAG = 6
EPS = 1e-5
QSCALE = (DH ** -0.5) * math.log2(math.e)
X_SPLIT = (0, 256, 512, 1280, 2048)
QUADS = ((0, 0), (0, 1), (1, 0), (1, 1))


def _layernorm(x):
    xc = x - jnp.mean(x, axis=-1, keepdims=True)
    v = jnp.mean(xc * xc, axis=-1, keepdims=True)
    return xc * lax.rsqrt(v + EPS)


def _layernorm_twice(x):
    xc = x - jnp.mean(x, axis=-1, keepdims=True)
    v = jnp.mean(xc * xc, axis=-1, keepdims=True)
    r = lax.rsqrt(v + EPS)
    return xc * (r * lax.rsqrt(v * r * r + EPS))


def _gelu(u):
    c = math.sqrt(2.0 / math.pi)
    z = u * (c + (c * 0.044715) * (u * u))
    hu = 0.5 * u
    return hu + hu * jnp.tanh(z)


def _dot(a, b):
    return jnp.dot(a, b, preferred_element_type=f32)


def _pack(a):
    return pltpu.bitcast(a.astype(bf16), u32)


def _unpack(w):
    return pltpu.bitcast(w, bf16)


def _lhs(ref, p):
    return jnp.concatenate([_unpack(ref[p, t]) for t in range(ref.shape[1])], axis=1)


def _after(x, t):
    t = jnp.tile(t, (x.shape[0] // t.shape[0], x.shape[1] // t.shape[1]))
    return jnp.maximum(x, jnp.minimum(x, t))


def _lhs_factors(a11, a12, a21, a22):
    return [a11 + a22, a21 + a22, a11, a22, a11 + a12, a21 - a11, a12 - a22]


def _rhs_factors(b11, b12, b21, b22):
    return [b11 + b22, b11, b12 - b22, b21 - b11, b22, b11 + b12, b21 + b22]


_RHS_TERMS = ((0, 3, 1), (0, None, 0), (1, 3, -1), (2, 0, -1), (3, None, 0), (0, 1, 1), (2, 3, 1))


def _combine(prod, first=()):
    done = {p: prod(p) for p in first}

    def m(p):
        return done[p] if p in done else prod(p)

    m0 = m(0)
    c11 = m0 + m(6)
    m3 = m(3)
    c11 = c11 + m3
    m4 = m(4)
    c11 = c11 - m4
    m2 = m(2)
    c12 = m2 + m4
    c22 = m0 + m2
    m1 = m(1)
    c21 = m1 + m3
    c22 = (c22 - m1) + m(5)
    return c11, c12, c21, c22


def _lhs_factors2(a):
    outer = [_lhs_factors(a[r][c], a[r][2 + c], a[2 + r][c], a[2 + r][2 + c]) for r, c in QUADS]
    return [v for p in range(7) for v in _lhs_factors(*(outer[q][p] for q in range(4)))]


class _Quad:
    def __init__(self, v):
        self.v = v

    def __add__(self, o):
        return _Quad([a + b for a, b in zip(self.v, o.v)])

    def __sub__(self, o):
        return _Quad([a - b for a, b in zip(self.v, o.v)])


def _combine2(prod, first=()):
    out = _combine(lambda p: _Quad(_combine(lambda q: prod(7 * p + q))), first)
    c = [[None] * 4 for _ in range(4)]
    for po, (ro, co) in enumerate(QUADS):
        for q, (r, cc) in enumerate(QUADS):
            c[2 * ro + r][2 * co + cc] = out[po].v[q]
    return c


def _projections(x_hbm, wqkv_hbm, late_copies, x_s, qT_s, k_s, vT_s, sem_x, sem_k, sem_w,
                 wk_s, wq_s, wv_s, wkb_s, wqb_s, wvb_s, y_s):
    copies = {}
    for i in range(len(X_SPLIT) - 1):
        rows = pl.ds(X_SPLIT[i], X_SPLIT[i + 1] - X_SPLIT[i])
        copies[f"x{i}"] = pltpu.make_async_copy(x_hbm.at[0, rows, :], x_s.at[rows, :], sem_x.at[i])
    for j in range(4):
        copies[f"k{j}"] = pltpu.make_async_copy(
            wqkv_hbm.at[:, pl.ds(D + j * 256, 256)], wk_s.at[j], sem_k.at[j])
    copies["q"] = pltpu.make_async_copy(wqkv_hbm.at[:, pl.ds(0, D)], wq_s, sem_w.at[0])
    copies["v"] = pltpu.make_async_copy(wqkv_hbm.at[:, pl.ds(2 * D, D)], wv_s, sem_w.at[1])

    start_after = {"x0": ("k2",), "k0": ("k3",), "k1": ("x1",), "k2": ("x2",), "x1": ("q", "v"), "x2": ("x3",)}

    def wait(tag):
        copies[tag].wait()
        for t in start_after.get(tag, ()):
            copies[t].start()

    for t in ("x0", "k0", "k1"):
        copies[t].start()

    def ln_piece(i, p, dep=None):
        r = p * 8
        x0 = x_s[i * QB + r:i * QB + r + 8, :].astype(f32)
        x1 = x_s[i * QB + 128 + r:i * QB + 128 + r + 8, :].astype(f32)
        if dep is not None:
            x0 = jnp.concatenate([_after(x0[:, :128], dep), x0[:, 128:]], axis=1)
            x1 = jnp.concatenate([_after(x1[:, :128], dep), x1[:, 128:]], axis=1)
        y0, y1 = _layernorm(x0), _layernorm(x1)
        for n, a in enumerate(_lhs_factors(y0[:, :D2], y0[:, D2:], y1[:, :D2], y1[:, D2:])):
            y_s[n, i * 128 + r:i * 128 + r + 8, :] = a.astype(bf16)

    def weight_sums(src, dst, j, r, dep=None):
        top, bot = src[r:r + 16, :].astype(f32), src[D2 + r:D2 + r + 16, :].astype(f32)
        b11, b12, b21, b22 = top[:, :128], top[:, 128:], bot[:, :128], bot[:, 128:]
        if dep is not None:
            b11, b22 = _after(b11, dep), _after(b22, dep)
        for n, b in enumerate(_rhs_factors(b11, b12, b21, b22)):
            if n not in (1, 4):
                dst[j, n, r:r + 16, :] = b.astype(bf16)

    last = [None]

    def products(src, dst, j, rows, before=None):
        def prod(p):
            if before is not None:
                before()
            if p == 1:
                b = src[:D2, :128]
            elif p == 4:
                b = src[D2:, 128:]
            else:
                b = dst[j, p]
            last[0] = _dot(y_s[p, rows, :], b)
            return last[0]
        return prod

    wait("x0")
    for p in range(16):
        ln_piece(0, p)
    qv_jobs = [(w.at[:, pl.ds(j * 256, 256)], wb, j, r) for w, wb in ((wq_s, wqb_s), (wv_s, wvb_s))
               for j in range(4) for r in range(0, D2, 16)]
    for i in range(NQB):
        count = [0]
        ln_from = {0: 22, 1: 15, 4: 15}.get(i, 0)

        def side_work():
            d = count[0]
            count[0] += 1
            if i + 1 < NQB and d >= ln_from:
                n = 26 - ln_from
                for p in range((d - ln_from) * 16 // n, min(16, (d - ln_from + 1) * 16 // n)):
                    ln_piece(i + 1, p, last[0][(p % 4) * 32:(p % 4) * 32 + 8])
            n0 = (i - 4) * 28 + d - 15
            if n0 >= 0:
                for p in range(n0 * len(qv_jobs) // 96, min(len(qv_jobs), (n0 + 1) * len(qv_jobs) // 96)):
                    weight_sums(*qv_jobs[p], last[0][32 + 64 * (p % 2):32 + 64 * (p % 2) + 8])

        for j in range(4):
            if i == 0:
                wait(f"k{j}")
                if j == 3:
                    wait("x1")
                for r in range(0, D2, 16):
                    weight_sums(wk_s.at[j], wkb_s, j, r)
            if i == 1 and j == 2:
                wait("x2")
            if i == 4 and j == 2:
                wait("x3")
                wait("q")
                wait("v")
            c = _combine(products(wk_s.at[j], wkb_s, j, slice(i * 128, (i + 1) * 128), side_work),
                         first=(1, 4) if i == 0 else ())
            for (t, g), val in zip(QUADS, c):
                k_s[2 * j + g, i * 128 + t * 64:i * 128 + (t + 1) * 64, :] = _pack(val)

    def qv_step(it, carry):
        @pl.when(it == 0)
        def _():
            for copy in late_copies:
                copy.start()

        for i in (2 * it, 2 * it + 1):
            rows = pl.ds(pl.multiple_of(i * 128, 128), 128)
            for w, wb, dst, scale in ((wq_s, wqb_s, qT_s, QSCALE), (wv_s, wvb_s, vT_s, None)):
                for j in range(4):
                    c = _combine(products(w.at[:, pl.ds(j * 256, 256)], wb, j, rows))
                    for (t, g), val in zip(QUADS, c):
                        if scale is not None:
                            val = val * scale
                        dst[2 * i + t, (2 * j + g) * 64:(2 * j + g + 1) * 64, :] = pltpu.bitcast(
                            val.astype(bf16).T, u32)
        return carry

    lax.fori_loop(0, NQB // 2, qv_step, 0)


def _attention(wo_s, w1_s, w2_s, qT_s, k_s, vT_s, wob_s, w1b_s, w2b_s, s_a, s_b, oT_s):
    scores = (s_a, s_b)

    def qk_chunk(u, j, c, s_s, m):
        u = jnp.minimum(u, NU - 1)
        qb, h = u // H, u % H
        ws = []
        for t in range(2):
            parts = [jnp.zeros((16, 128), u32)] * 4
            parts[j] = qT_s[qb * 2 + t, pl.ds(pl.multiple_of(h * 16, 16), 16), :]
            ws.append(_unpack(jnp.concatenate(parts, axis=0)))
        keys = _unpack(k_s[h // 4, c * KC // 2:(c + 1) * KC // 2, :])
        s = _dot(keys, jnp.concatenate(ws, axis=1))
        s_s[c * KC:(c + 1) * KC, :] = s
        for r in range(0, KC, 8):
            m = s[r:r + 8] if m is None else jnp.maximum(m, s[r:r + 8])
        return m

    def row_max(m):
        return jnp.broadcast_to(jnp.max(m, axis=0, keepdims=True), (8, QB))

    def pv_chunk(u, c, s_s, mx, l, acc):
        h = u % H
        ps = []
        for r in range(c * KC, (c + 1) * KC, 16):
            p0 = jnp.exp2(s_s[r:r + 8, :] - mx)
            p1 = jnp.exp2(s_s[r + 8:r + 16, :] - mx)
            l = p0 + p1 if l is None else l + (p0 + p1)
            ps += [p0, p1]
        p = jnp.concatenate(ps, axis=0).astype(bf16)
        a = _dot(_unpack(vT_s[c, pl.ds(pl.multiple_of(h * 16, 16), 16), :]), p)
        return l, (a if acc is None else acc + a)

    def weight_jobs(it):
        jobs = []

        def two_level(src, dst, kq, nq, r0, n, p):
            outer = []

            def blk(r, c):
                return src[pl.ds(r * kq + r0, 16), c * nq + n * 128:c * nq + (n + 1) * 128].astype(f32)

            def emit(qs, dep):
                o = list(outer)
                if dep is not None:
                    o[0], o[3] = _after(o[0], dep), _after(o[3], dep)
                vals = _rhs_factors(*o)
                for q in qs:
                    dst[7 * p + q, n, pl.ds(pl.multiple_of(r0 // 2, 8), 8), :] = _pack(vals[q])

            def begin(dep):
                qa, qb, sign = _RHS_TERMS[p]
                for r, c in QUADS:
                    v = blk(2 * QUADS[qa][0] + r, 2 * QUADS[qa][1] + c)
                    if r == c:
                        v = _after(v, dep)
                    if sign:
                        v2 = blk(2 * QUADS[qb][0] + r, 2 * QUADS[qb][1] + c)
                        v = v + v2 if sign > 0 else v - v2
                    outer.append(v)
                emit(range(3), None)

            jobs.append(begin)
            jobs.append(lambda dep: emit(range(3, 7), dep))

        def one_level(r0, j):
            def run(dep):
                top = _after(wo_s[pl.ds(r0, 16), j * 256:(j + 1) * 256].astype(f32), dep)
                bot = wo_s[pl.ds(D2 + r0, 16), j * 256:(j + 1) * 256].astype(f32)
                for n, b in enumerate(_rhs_factors(top[:, :128], top[:, 128:], bot[:, :128], bot[:, 128:])):
                    wob_s[j, n, pl.ds(pl.multiple_of(r0 // 2, 8), 8), :] = _pack(b)
            jobs.append(run)

        def row_groups(total):
            per_step = -(-(total // 16) // NIT)
            return [pl.multiple_of(jnp.minimum(it * per_step + a, total // 16 - 1) * 16, 16)
                    for a in range(per_step)]

        for src, dst, kq, nq in ((w1_s, w1b_s, D4, F4), (w2_s, w2b_s, F4, D4)):
            for r0 in row_groups(kq):
                for n in range(nq // 128):
                    for p in range(7):
                        two_level(src, dst, kq, nq, r0, n, p)
        for r0 in row_groups(D2):
            for j in range(4):
                one_level(r0, j)
        return jobs

    def unit(it, j, mx, m, hist, jobs):
        u = UNROLL * it + j
        l = acc = mx_next = None
        for c in range(NC):
            cq = c + SKEW
            if cq < NC:
                m = qk_chunk(u + 1, (j + 1) % 4, cq, scores[(j + 1) % 2], m)
                if cq == NC - 1:
                    mx_next, m = row_max(m), None
            else:
                m = qk_chunk(u + 2, (j + 2) % 4, cq - NC, scores[j % 2], m)
            hist.append(m if m is not None else mx_next)
            n0, n1 = j * NC + c, UNROLL * NC
            for p in range(n0 * len(jobs) // n1, (n0 + 1) * len(jobs) // n1):
                jobs[p](hist[-1][:, :128])
            mxc = _after(mx, hist[-LAG]) if len(hist) >= LAG else mx
            l, acc = pv_chunk(u, c, scores[j % 2], mxc, l, acc)
        o = acc * (1.0 / jnp.sum(l, axis=0, keepdims=True))
        for t in range(2):
            oT_s[(u // H) * 2 + t, pl.ds(pl.multiple_of((u % H) * DH, DH), DH), :] = o[:, t * 128:(t + 1) * 128]
        return mx_next, m

    m = None
    for c in range(NC):
        m = qk_chunk(0, 0, c, s_a, m)
    mx, m = row_max(m), None
    for c in range(SKEW):
        m = qk_chunk(1, 1, c, s_b, m)

    def step(it, carry):
        mx, m = carry
        hist = []
        jobs = weight_jobs(it)
        for j in range(UNROLL):
            mx, m = unit(it, j, mx, m, hist, jobs)
        return mx, m

    lax.fori_loop(0, NIT, step, (mx, m))


def _mix(b1_ref, b2_ref, out_hbm, x_s, sem_o, wob_s, w1b_s, w2b_s, oT_s, oa_s, h_s, y0_s, ya_s, ua_s, out_s):
    def out_copy(qb, slot):
        return pltpu.make_async_copy(
            out_s.at[slot], out_hbm.at[0, pl.ds(pl.multiple_of(qb * QB, QB), QB), :], sem_o.at[slot])

    def o_factors(qb, t, g, dep=None):
        lo = oT_s[2 * qb + t, g * 128:(g + 1) * 128, :]
        hi = oT_s[2 * qb + t, D2 + g * 128:D2 + (g + 1) * 128, :]
        if dep is not None:
            lo, hi = _after(lo, dep), _after(hi, dep)
        lo, hi = lo.T, hi.T
        for n, a in enumerate(_lhs_factors(lo[:64], hi[:64], lo[64:], hi[64:])):
            oa_s[7 * t + n, g] = _pack(a)

    def blocks(ys, kt):
        return [[y[:, cq * D4 + kt * 128:cq * D4 + (kt + 1) * 128] for cq in range(4)] for y in ys]

    def step(qb, carry):
        slot = qb % 2

        @pl.when(qb >= 2)
        def _():
            out_copy(qb - 2, slot).wait()

        b1 = b1_ref[...].astype(f32).reshape(1, F)
        b2 = b2_ref[...].astype(f32).reshape(1, D)
        r0 = pl.multiple_of(qb * QB, QB)

        for t in range(2):
            for j in range(4):
                c = _combine(lambda p: _dot(_lhs(oa_s, 7 * t + p), _unpack(wob_s[j, p])))
                for (r, g), val in zip(QUADS, c):
                    cs = slice((2 * j + g) * 128, (2 * j + g + 1) * 128)
                    ro = t * 128 + r * 64
                    h_s[ro:ro + 64, cs] = x_s[pl.ds(r0 + ro, 64), cs].astype(f32) + val
            for r in range(0, 64, 16):
                ys = [_layernorm_twice(h_s[t * 128 + q * 64 + r:t * 128 + q * 64 + r + 16, :]) for q in range(2)]
                if t == 0:
                    for q in range(2):
                        y0_s[q * 64 + r:q * 64 + r + 16, :] = ys[q]
                    for kt in range(2):
                        a = blocks(ys, kt)
                        top = [(a[q][cc], a[q][cc] + a[q][2 + cc]) for q, cc in QUADS]
                        for p, sel in ((2, 0), (4, 1)):
                            for n, v in enumerate(_lhs_factors(*(o[sel] for o in top))):
                                ya_s[7 * p + n, kt, r // 2:r // 2 + 8, :] = _pack(v)
                else:
                    ys = [y0_s[q * 64 + r:q * 64 + r + 16, :] for q in range(2)] + ys
                    for kt in range(2):
                        for n, v in enumerate(_lhs_factors2(blocks(ys, kt))):
                            if n // 7 not in (2, 4):
                                ya_s[n, kt, r // 2:r // 2 + 8, :] = _pack(v)

        for n in range(F4 // 128):
            c = _combine2(lambda p: _dot(_lhs(ya_s, p), _unpack(w1b_s[p, n])), first=(2, 4) if n == 0 else ())
            for r in range(0, 64, 16):
                u = [[_gelu(c[t][cq][r:r + 16] + b1[:, cq * F4 + n * 128:cq * F4 + (n + 1) * 128])
                      for cq in range(4)] for t in range(4)]
                for p, a in enumerate(_lhs_factors2(u)):
                    ua_s[p, n, r // 2:r // 2 + 8, :] = _pack(a)

        nxt = jnp.minimum(qb + 1, NQB - 1)
        for n in range(D4 // 128):
            count = [0]

            def prod(p):
                val = _dot(_lhs(ua_s, p), _unpack(w2b_s[p, n]))
                if count[0] % 12 == 2:
                    o_factors(nxt, n, count[0] // 12, val[:8])
                count[0] += 1
                return val

            c = _combine2(prod)
            for t in range(4):
                for cq in range(4):
                    rs, cs = slice(t * 64, (t + 1) * 64), slice(cq * D4 + n * 128, cq * D4 + (n + 1) * 128)
                    out_s[slot, rs, cs] = (h_s[rs, cs] + (c[t][cq] + b2[:, cs])).astype(bf16)
        out_copy(qb, slot).start()
        return carry

    for t in range(2):
        for g in range(4):
            o_factors(0, t, g)
    lax.fori_loop(0, NQB, step, 0)
    out_copy(NQB - 2, 0).wait()
    out_copy(NQB - 1, 1).wait()


def _kernel(x_hbm, wqkv_hbm, wo_hbm, w1_hbm, b1_ref, w2_hbm, b2_ref, out_hbm,
            x_s, wo_s, w1_s, w2_s, qT_s, k_s, vT_s, sem_x, sem_k, sem_w, sem_o):
    late_copies = (pltpu.make_async_copy(w1_hbm, w1_s, sem_w.at[2]),
                   pltpu.make_async_copy(w2_hbm, w2_s, sem_w.at[3]),
                   pltpu.make_async_copy(wo_hbm, wo_s, sem_w.at[4]))

    def first(*bufs):
        _projections(x_hbm, wqkv_hbm, late_copies, x_s, qT_s, k_s, vT_s, sem_x, sem_k, sem_w, *bufs)

    pl.run_scoped(
        first,
        pltpu.VMEM((4, D, 256), bf16),
        pltpu.VMEM((D, D), bf16),
        pltpu.VMEM((D, D), bf16),
        pltpu.VMEM((4, 7, D2, 128), bf16),
        pltpu.VMEM((4, 7, D2, 128), bf16),
        pltpu.VMEM((4, 7, D2, 128), bf16),
        pltpu.VMEM((7, S // 2, D2), bf16))

    def second(wob_s, w1b_s, w2b_s, s_a, s_b, oT_s, *bufs):
        for copy in late_copies:
            copy.wait()
        _attention(wo_s, w1_s, w2_s, qT_s, k_s, vT_s, wob_s, w1b_s, w2b_s, s_a, s_b, oT_s)
        _mix(b1_ref, b2_ref, out_hbm, x_s, sem_o, wob_s, w1b_s, w2b_s, oT_s, *bufs)

    pl.run_scoped(
        second,
        pltpu.VMEM((4, 7, D2 // 2, 128), u32),
        pltpu.VMEM((49, F4 // 128, D4 // 2, 128), u32),
        pltpu.VMEM((49, D4 // 128, F4 // 2, 128), u32),
        pltpu.VMEM((S, QB), f32),
        pltpu.VMEM((S, QB), f32),
        pltpu.VMEM((S // 128, D, 128), f32),
        pltpu.VMEM((14, 4, 32, 128), u32),
        pltpu.VMEM((QB, D), f32),
        pltpu.VMEM((128, D), f32),
        pltpu.VMEM((49, D4 // 128, 32, 128), u32),
        pltpu.VMEM((49, F4 // 128, 32, 128), u32),
        pltpu.VMEM((2, QB, D), bf16))


@jax.jit
def pallas_sequential_preLN__softmax_full_mha__mixer_channel_mlp__prompt_kernel(
    A_x: jax.Array,
    A_wqkv: jax.Array,
    A_wo: jax.Array,
    B_x: jax.Array,
    B_w1: jax.Array,
    B_b1: jax.Array,
    B_w2: jax.Array,
    B_b2: jax.Array,
):
    del B_x
    hbm = pl.BlockSpec(memory_space=pl.ANY)
    vmem = pl.BlockSpec(memory_space=pltpu.VMEM)
    return pl.pallas_call(
        _kernel,
        out_shape=jax.ShapeDtypeStruct((1, S, D), bf16),
        in_specs=[hbm, hbm, hbm, hbm, vmem, hbm, vmem],
        out_specs=hbm,
        scratch_shapes=[
            pltpu.VMEM((S, D), bf16),
            pltpu.VMEM((D, D), bf16),
            pltpu.VMEM((D, F), bf16),
            pltpu.VMEM((F, D), bf16),
            pltpu.VMEM((S // 128, D2, 128), u32),
            pltpu.VMEM((8, S // 2, 128), u32),
            pltpu.VMEM((S // 128, D2, 128), u32),
            pltpu.SemaphoreType.DMA((len(X_SPLIT) - 1,)),
            pltpu.SemaphoreType.DMA((4,)),
            pltpu.SemaphoreType.DMA((5,)),
            pltpu.SemaphoreType.DMA((2,)),
        ],
        compiler_params=pltpu.CompilerParams(vmem_limit_bytes=120 << 20),
    )(A_x, A_wqkv, A_wo, B_w1, B_b1, B_w2, B_b2)
```

```python
import math

import jax
import jax.numpy as jnp
from jax import lax
from jax.experimental import pallas as pl
from jax.experimental.pallas import tpu as pltpu

f32, bf16, u32 = jnp.float32, jnp.bfloat16, jnp.uint32

S, D, H, DH, F = 2048, 1024, 32, 32, 3584
D2, D4, F4 = D // 2, D // 4, F // 4
QB = 256
NQB = S // QB
KC = 128
NC = S // KC
NU = NQB * H
UNROLL = 16
NIT = NU // UNROLL
SKEW = 4
LAG = 6
EPS = 1e-5
QSCALE = (DH ** -0.5) * math.log2(math.e)
X_SPLIT = (0, 256, 512, 1280, 2048)
QUADS = ((0, 0), (0, 1), (1, 0), (1, 1))


def _layernorm(x):
    xc = x - jnp.mean(x, axis=-1, keepdims=True)
    v = jnp.mean(xc * xc, axis=-1, keepdims=True)
    return xc * lax.rsqrt(v + EPS)


def _layernorm_twice(x):
    xc = x - jnp.mean(x, axis=-1, keepdims=True)
    v = jnp.mean(xc * xc, axis=-1, keepdims=True)
    r = lax.rsqrt(v + EPS)
    return xc * (r * lax.rsqrt(v * r * r + EPS))


def _gelu(u):
    c = math.sqrt(2.0 / math.pi)
    z = u * (c + (c * 0.044715) * (u * u))
    hu = 0.5 * u
    return hu + hu * jnp.tanh(z)


def _dot(a, b):
    return jnp.dot(a, b, preferred_element_type=f32)


def _pack(a):
    return pltpu.bitcast(a.astype(bf16), u32)


def _unpack(w):
    return pltpu.bitcast(w, bf16)


def _lhs(ref, p):
    return jnp.concatenate([_unpack(ref[p, t]) for t in range(ref.shape[1])], axis=1)


def _after(x, t):
    t = jnp.tile(t, (x.shape[0] // t.shape[0], x.shape[1] // t.shape[1]))
    return jnp.maximum(x, jnp.minimum(x, t))


def _lhs_factors(a11, a12, a21, a22):
    return [a11 + a22, a21 + a22, a11, a22, a11 + a12, a21 - a11, a12 - a22]


def _rhs_factors(b11, b12, b21, b22):
    return [b11 + b22, b11, b12 - b22, b21 - b11, b22, b11 + b12, b21 + b22]


_RHS_TERMS = ((0, 3, 1), (0, None, 0), (1, 3, -1), (2, 0, -1), (3, None, 0), (0, 1, 1), (2, 3, 1))


def _combine(prod, first=()):
    done = {p: prod(p) for p in first}

    def m(p):
        return done[p] if p in done else prod(p)

    m0 = m(0)
    c11 = m0 + m(6)
    m3 = m(3)
    c11 = c11 + m3
    m4 = m(4)
    c11 = c11 - m4
    m2 = m(2)
    c12 = m2 + m4
    c22 = m0 + m2
    m1 = m(1)
    c21 = m1 + m3
    c22 = (c22 - m1) + m(5)
    return c11, c12, c21, c22


def _lhs_factors2(a):
    outer = [_lhs_factors(a[r][c], a[r][2 + c], a[2 + r][c], a[2 + r][2 + c]) for r, c in QUADS]
    return [v for p in range(7) for v in _lhs_factors(*(outer[q][p] for q in range(4)))]


class _Quad:
    def __init__(self, v):
        self.v = v

    def __add__(self, o):
        return _Quad([a + b for a, b in zip(self.v, o.v)])

    def __sub__(self, o):
        return _Quad([a - b for a, b in zip(self.v, o.v)])


def _inner(prod, p):
    return _Quad(_combine(lambda q: prod(7 * p + q)))


def _combine2(outer):
    out = _combine(outer)
    c = [[None] * 4 for _ in range(4)]
    for po, (ro, co) in enumerate(QUADS):
        for q, (r, cc) in enumerate(QUADS):
            c[2 * ro + r][2 * co + cc] = out[po].v[q]
    return c


def _projections(x_hbm, wqkv_hbm, late_copies, x_s, qT_s, k_s, vT_s, sem_x, sem_k, sem_w,
                 wk_s, wq_s, wv_s, wkb_s, wqb_s, wvb_s, y_s):
    copies = {}
    for i in range(len(X_SPLIT) - 1):
        rows = pl.ds(X_SPLIT[i], X_SPLIT[i + 1] - X_SPLIT[i])
        copies[f"x{i}"] = pltpu.make_async_copy(x_hbm.at[0, rows, :], x_s.at[rows, :], sem_x.at[i])
    for j in range(4):
        copies[f"k{j}"] = pltpu.make_async_copy(
            wqkv_hbm.at[:, pl.ds(D + j * 256, 256)], wk_s.at[j], sem_k.at[j])
    copies["q"] = pltpu.make_async_copy(wqkv_hbm.at[:, pl.ds(0, D)], wq_s, sem_w.at[0])
    copies["v"] = pltpu.make_async_copy(wqkv_hbm.at[:, pl.ds(2 * D, D)], wv_s, sem_w.at[1])

    start_after = {"x0": ("k2",), "k0": ("k3",), "k1": ("x1",), "k2": ("x2",), "x1": ("q", "v"), "x2": ("x3",)}

    def wait(tag):
        copies[tag].wait()
        for t in start_after.get(tag, ()):
            copies[t].start()

    for t in ("x0", "k0", "k1"):
        copies[t].start()

    def ln_piece(i, p, dep=None):
        r = p * 8
        x0 = x_s[i * QB + r:i * QB + r + 8, :].astype(f32)
        x1 = x_s[i * QB + 128 + r:i * QB + 128 + r + 8, :].astype(f32)
        if dep is not None:
            x0 = jnp.concatenate([_after(x0[:, :128], dep), x0[:, 128:]], axis=1)
            x1 = jnp.concatenate([_after(x1[:, :128], dep), x1[:, 128:]], axis=1)
        y0, y1 = _layernorm(x0), _layernorm(x1)
        for n, a in enumerate(_lhs_factors(y0[:, :D2], y0[:, D2:], y1[:, :D2], y1[:, D2:])):
            y_s[n, i * 128 + r:i * 128 + r + 8, :] = a.astype(bf16)

    def weight_sums(src, dst, j, r, dep=None):
        top, bot = src[r:r + 16, :].astype(f32), src[D2 + r:D2 + r + 16, :].astype(f32)
        b11, b12, b21, b22 = top[:, :128], top[:, 128:], bot[:, :128], bot[:, 128:]
        if dep is not None:
            b11, b22 = _after(b11, dep), _after(b22, dep)
        for n, b in enumerate(_rhs_factors(b11, b12, b21, b22)):
            if n not in (1, 4):
                dst[j, n, r:r + 16, :] = b.astype(bf16)

    last = [None]

    def products(src, dst, j, rows, before=None):
        def prod(p):
            if before is not None:
                before()
            if p == 1:
                b = src[:D2, :128]
            elif p == 4:
                b = src[D2:, 128:]
            else:
                b = dst[j, p]
            last[0] = _dot(y_s[p, rows, :], b)
            return last[0]
        return prod

    def sum_jobs(w, wb):
        return [(w.at[:, pl.ds(j * 256, 256)], wb, j, r) for j in range(4) for r in range(0, D2, 16)]

    wait("x0")
    for p in range(16):
        ln_piece(0, p)
    q_jobs = sum_jobs(wq_s, wqb_s)
    for i in range(NQB):
        count = [0]
        ln_from = {0: 22, 1: 15, 4: 15}.get(i, 0)

        def side_work():
            d = count[0]
            count[0] += 1
            if i + 1 < NQB and d >= ln_from:
                n = 26 - ln_from
                for p in range((d - ln_from) * 16 // n, min(16, (d - ln_from + 1) * 16 // n)):
                    ln_piece(i + 1, p, last[0][(p % 4) * 32:(p % 4) * 32 + 8])
            n0 = (i - 4) * 28 + d - 15
            if n0 >= 0:
                for p in range(n0 * len(q_jobs) // 96, min(len(q_jobs), (n0 + 1) * len(q_jobs) // 96)):
                    weight_sums(*q_jobs[p], last[0][32 + 64 * (p % 2):32 + 64 * (p % 2) + 8])

        for j in range(4):
            if i == 0:
                wait(f"k{j}")
                if j == 3:
                    wait("x1")
                for r in range(0, D2, 16):
                    weight_sums(wk_s.at[j], wkb_s, j, r)
            if i == 1 and j == 2:
                wait("x2")
            if i == 4 and j == 2:
                wait("x3")
                wait("q")
                wait("v")
            c = _combine(products(wk_s.at[j], wkb_s, j, slice(i * 128, (i + 1) * 128), side_work),
                         first=(1, 4) if i == 0 else ())
            for (t, g), val in zip(QUADS, c):
                k_s[2 * j + g, i * 128 + t * 64:i * 128 + (t + 1) * 64, :] = _pack(val)

    for copy in late_copies:
        copy.start()
    for w, wb, dst, scale, jobs in ((wq_s, wqb_s, qT_s, QSCALE, sum_jobs(wv_s, wvb_s)),
                                    (wv_s, wvb_s, vT_s, None, [])):
        def next_job():
            if jobs:
                weight_sums(*jobs.pop(0), last[0][32:40])

        for i in range(NQB):
            for j in range(4):
                c = _combine(products(w.at[:, pl.ds(j * 256, 256)], wb, j, slice(i * 128, (i + 1) * 128), next_job))
                for (t, g), val in zip(QUADS, c):
                    if scale is not None:
                        val = val * scale
                    dst[2 * i + t, (2 * j + g) * 64:(2 * j + g + 1) * 64, :] = pltpu.bitcast(
                        val.astype(bf16).T, u32)


def _attention(late_copies, wo_s, w1_s, w2_s, qT_s, k_s, vT_s, wob_s, w1b_s, w2b_s, s_a, s_b, oT_s):
    scores = (s_a, s_b)

    def qk_chunk(u, j, c, s_s, m):
        u = jnp.minimum(u, NU - 1)
        qb, h = u // H, u % H
        ws = []
        for t in range(2):
            parts = [jnp.zeros((16, 128), u32)] * 4
            parts[j] = qT_s[qb * 2 + t, pl.ds(pl.multiple_of(h * 16, 16), 16), :]
            ws.append(_unpack(jnp.concatenate(parts, axis=0)))
        keys = _unpack(k_s[h // 4, c * KC // 2:(c + 1) * KC // 2, :])
        s = _dot(keys, jnp.concatenate(ws, axis=1))
        s_s[c * KC:(c + 1) * KC, :] = s
        for r in range(0, KC, 8):
            m = s[r:r + 8] if m is None else jnp.maximum(m, s[r:r + 8])
        return m

    def row_max(m):
        return jnp.broadcast_to(jnp.max(m, axis=0, keepdims=True), (8, QB))

    def pv_chunk(u, c, s_s, mx, l, acc):
        h = u % H
        ps = []
        for r in range(c * KC, (c + 1) * KC, 16):
            p0 = jnp.exp2(s_s[r:r + 8, :] - mx)
            p1 = jnp.exp2(s_s[r + 8:r + 16, :] - mx)
            l = p0 + p1 if l is None else l + (p0 + p1)
            ps += [p0, p1]
        p = jnp.concatenate(ps, axis=0).astype(bf16)
        a = _dot(_unpack(vT_s[c, pl.ds(pl.multiple_of(h * 16, 16), 16), :]), p)
        return l, (a if acc is None else acc + a)

    def weight_jobs(it):
        jobs = []

        def two_level(src, dst, kq, nq, r0, n, p):
            outer = []

            def blk(r, c):
                return src[pl.ds(r * kq + r0, 16), c * nq + n * 128:c * nq + (n + 1) * 128].astype(f32)

            def emit(qs, dep):
                o = list(outer)
                if dep is not None:
                    o[0], o[3] = _after(o[0], dep), _after(o[3], dep)
                vals = _rhs_factors(*o)
                for q in qs:
                    dst[7 * p + q, n, pl.ds(pl.multiple_of(r0 // 2, 8), 8), :] = _pack(vals[q])

            def begin(dep):
                qa, qb, sign = _RHS_TERMS[p]
                for r, c in QUADS:
                    v = blk(2 * QUADS[qa][0] + r, 2 * QUADS[qa][1] + c)
                    if r == c:
                        v = _after(v, dep)
                    if sign:
                        v2 = blk(2 * QUADS[qb][0] + r, 2 * QUADS[qb][1] + c)
                        v = v + v2 if sign > 0 else v - v2
                    outer.append(v)
                emit(range(3), None)

            jobs.append(begin)
            jobs.append(lambda dep: emit(range(3, 7), dep))

        def one_level(r0, j):
            def run(dep):
                top = _after(wo_s[pl.ds(r0, 16), j * 256:(j + 1) * 256].astype(f32), dep)
                bot = wo_s[pl.ds(D2 + r0, 16), j * 256:(j + 1) * 256].astype(f32)
                for n, b in enumerate(_rhs_factors(top[:, :128], top[:, 128:], bot[:, :128], bot[:, 128:])):
                    wob_s[j, n, pl.ds(pl.multiple_of(r0 // 2, 8), 8), :] = _pack(b)
            jobs.append(run)

        def row_groups(total):
            per_step = -(-(total // 16) // NIT)
            return [pl.multiple_of(jnp.minimum(it * per_step + a, total // 16 - 1) * 16, 16)
                    for a in range(per_step)]

        for src, dst, kq, nq in ((w1_s, w1b_s, D4, F4), (w2_s, w2b_s, F4, D4)):
            for r0 in row_groups(kq):
                for n in range(nq // 128):
                    for p in range(7):
                        two_level(src, dst, kq, nq, r0, n, p)
        for r0 in row_groups(D2):
            for j in range(4):
                one_level(r0, j)
        return jobs

    def unit(it, j, mx, m, hist, jobs):
        u = UNROLL * it + j
        l = acc = mx_next = None
        for c in range(NC):
            cq = c + SKEW
            if cq < NC:
                m = qk_chunk(u + 1, (j + 1) % 4, cq, scores[(j + 1) % 2], m)
                if cq == NC - 1:
                    mx_next, m = row_max(m), None
            else:
                m = qk_chunk(u + 2, (j + 2) % 4, cq - NC, scores[j % 2], m)
            hist.append(m if m is not None else mx_next)
            n0, n1 = j * NC + c, UNROLL * NC
            for p in range(n0 * len(jobs) // n1, (n0 + 1) * len(jobs) // n1):
                jobs[p](hist[-1][:, :128])
            mxc = _after(mx, hist[-LAG]) if len(hist) >= LAG else mx
            l, acc = pv_chunk(u, c, scores[j % 2], mxc, l, acc)
        o = acc * (1.0 / jnp.sum(l, axis=0, keepdims=True))
        for t in range(2):
            oT_s[(u // H) * 2 + t, pl.ds(pl.multiple_of((u % H) * DH, DH), DH), :] = o[:, t * 128:(t + 1) * 128]
        return mx_next, m

    m = None
    for c in range(NC):
        m = qk_chunk(0, 0, c, s_a, m)
    mx, m = row_max(m), None
    for c in range(SKEW):
        m = qk_chunk(1, 1, c, s_b, m)
    for copy in late_copies:
        copy.wait()

    def step(it, carry):
        mx, m = carry
        hist = []
        jobs = weight_jobs(it)
        for j in range(UNROLL):
            mx, m = unit(it, j, mx, m, hist, jobs)
        return mx, m

    lax.fori_loop(0, NIT, step, (mx, m))


def _mix(b1_ref, b2_ref, out_hbm, x_s, sem_o, wob_s, w1b_s, w2b_s, oT_s, oa_s, h_s, y0_s, ya_s, ua_s, out_s):
    def out_copy(qb, slot):
        return pltpu.make_async_copy(
            out_s.at[slot], out_hbm.at[0, pl.ds(pl.multiple_of(qb * QB, QB), QB), :], sem_o.at[slot])

    def o_factors(qb, t, g, dep=None):
        lo = oT_s[2 * qb + t, g * 128:(g + 1) * 128, :]
        hi = oT_s[2 * qb + t, D2 + g * 128:D2 + (g + 1) * 128, :]
        if dep is not None:
            lo, hi = _after(lo, dep), _after(hi, dep)
        lo, hi = lo.T, hi.T
        for n, a in enumerate(_lhs_factors(lo[:64], hi[:64], lo[64:], hi[64:])):
            oa_s[7 * t + n, g] = _pack(a)

    def blocks(ys, kt):
        return [[y[:, cq * D4 + kt * 128:cq * D4 + (kt + 1) * 128] for cq in range(4)] for y in ys]

    def step(qb, carry):
        slot = qb % 2

        @pl.when(qb >= 2)
        def _():
            out_copy(qb - 2, slot).wait()

        b1 = b1_ref[...].astype(f32).reshape(1, F)
        b2 = b2_ref[...].astype(f32).reshape(1, D)
        r0 = pl.multiple_of(qb * QB, QB)

        for t in range(2):
            for j in range(4):
                c = _combine(lambda p: _dot(_lhs(oa_s, 7 * t + p), _unpack(wob_s[j, p])))
                for (r, g), val in zip(QUADS, c):
                    cs = slice((2 * j + g) * 128, (2 * j + g + 1) * 128)
                    ro = t * 128 + r * 64
                    h_s[ro:ro + 64, cs] = x_s[pl.ds(r0 + ro, 64), cs].astype(f32) + val
            for r in range(0, 64, 16):
                ys = [_layernorm_twice(h_s[t * 128 + q * 64 + r:t * 128 + q * 64 + r + 16, :]) for q in range(2)]
                if t == 0:
                    for q in range(2):
                        y0_s[q * 64 + r:q * 64 + r + 16, :] = ys[q]
                    for kt in range(2):
                        a = blocks(ys, kt)
                        top = [(a[q][cc], a[q][cc] + a[q][2 + cc]) for q, cc in QUADS]
                        for p, sel in ((2, 0), (4, 1)):
                            for n, v in enumerate(_lhs_factors(*(o[sel] for o in top))):
                                ya_s[7 * p + n, kt, r // 2:r // 2 + 8, :] = _pack(v)
                else:
                    ys = [y0_s[q * 64 + r:q * 64 + r + 16, :] for q in range(2)] + ys
                    for kt in range(2):
                        for n, v in enumerate(_lhs_factors2(blocks(ys, kt))):
                            if n // 7 not in (2, 4):
                                ya_s[n, kt, r // 2:r // 2 + 8, :] = _pack(v)

        def up(n, p):
            return _inner(lambda q: _dot(_lhs(ya_s, q), _unpack(w1b_s[q, n])), p)

        ahead = {(n, p): up(n, p) for n in range(2) for p in (2, 4)}
        for n in range(F4 // 128):
            c = _combine2(lambda p: ahead[n, p] if (n, p) in ahead else up(n, p))
            for r in range(0, 64, 16):
                u = [[_gelu(c[t][cq][r:r + 16] + b1[:, cq * F4 + n * 128:cq * F4 + (n + 1) * 128])
                      for cq in range(4)] for t in range(4)]
                for p, a in enumerate(_lhs_factors2(u)):
                    ua_s[p, n, r // 2:r // 2 + 8, :] = _pack(a)

        nxt = jnp.minimum(qb + 1, NQB - 1)
        for n in range(D4 // 128):
            count = [0]

            def prod(p):
                val = _dot(_lhs(ua_s, p), _unpack(w2b_s[p, n]))
                if count[0] % 12 == 8:
                    o_factors(nxt, n, count[0] // 12, val[:8])
                count[0] += 1
                return val

            c = _combine2(lambda p: _inner(prod, p))
            for t in range(4):
                for cq in range(4):
                    rs, cs = slice(t * 64, (t + 1) * 64), slice(cq * D4 + n * 128, cq * D4 + (n + 1) * 128)
                    out_s[slot, rs, cs] = (h_s[rs, cs] + (c[t][cq] + b2[:, cs])).astype(bf16)
        out_copy(qb, slot).start()
        return carry

    for t in range(2):
        for g in range(4):
            o_factors(0, t, g)
    lax.fori_loop(0, NQB, step, 0)
    out_copy(NQB - 2, 0).wait()
    out_copy(NQB - 1, 1).wait()


def _kernel(x_hbm, wqkv_hbm, wo_hbm, w1_hbm, b1_ref, w2_hbm, b2_ref, out_hbm,
            x_s, wo_s, w1_s, w2_s, qT_s, k_s, vT_s, sem_x, sem_k, sem_w, sem_o):
    late_copies = (pltpu.make_async_copy(w1_hbm, w1_s, sem_w.at[2]),
                   pltpu.make_async_copy(w2_hbm, w2_s, sem_w.at[3]),
                   pltpu.make_async_copy(wo_hbm, wo_s, sem_w.at[4]))

    def first(*bufs):
        _projections(x_hbm, wqkv_hbm, late_copies, x_s, qT_s, k_s, vT_s, sem_x, sem_k, sem_w, *bufs)

    pl.run_scoped(
        first,
        pltpu.VMEM((4, D, 256), bf16),
        pltpu.VMEM((D, D), bf16),
        pltpu.VMEM((D, D), bf16),
        pltpu.VMEM((4, 7, D2, 128), bf16),
        pltpu.VMEM((4, 7, D2, 128), bf16),
        pltpu.VMEM((4, 7, D2, 128), bf16),
        pltpu.VMEM((7, S // 2, D2), bf16))

    def second(wob_s, w1b_s, w2b_s, s_a, s_b, oT_s, *bufs):
        _attention(late_copies, wo_s, w1_s, w2_s, qT_s, k_s, vT_s, wob_s, w1b_s, w2b_s, s_a, s_b, oT_s)
        _mix(b1_ref, b2_ref, out_hbm, x_s, sem_o, wob_s, w1b_s, w2b_s, oT_s, *bufs)

    pl.run_scoped(
        second,
        pltpu.VMEM((4, 7, D2 // 2, 128), u32),
        pltpu.VMEM((49, F4 // 128, D4 // 2, 128), u32),
        pltpu.VMEM((49, D4 // 128, F4 // 2, 128), u32),
        pltpu.VMEM((S, QB), f32),
        pltpu.VMEM((S, QB), f32),
        pltpu.VMEM((S // 128, D, 128), f32),
        pltpu.VMEM((14, 4, 32, 128), u32),
        pltpu.VMEM((QB, D), f32),
        pltpu.VMEM((128, D), f32),
        pltpu.VMEM((49, D4 // 128, 32, 128), u32),
        pltpu.VMEM((49, F4 // 128, 32, 128), u32),
        pltpu.VMEM((2, QB, D), bf16))


@jax.jit
def pallas_sequential_preLN__softmax_full_mha__mixer_channel_mlp__prompt_kernel(
    A_x: jax.Array,
    A_wqkv: jax.Array,
    A_wo: jax.Array,
    B_x: jax.Array,
    B_w1: jax.Array,
    B_b1: jax.Array,
    B_w2: jax.Array,
    B_b2: jax.Array,
):
    del B_x
    hbm = pl.BlockSpec(memory_space=pl.ANY)
    vmem = pl.BlockSpec(memory_space=pltpu.VMEM)
    return pl.pallas_call(
        _kernel,
        out_shape=jax.ShapeDtypeStruct((1, S, D), bf16),
        in_specs=[hbm, hbm, hbm, hbm, vmem, hbm, vmem],
        out_specs=hbm,
        scratch_shapes=[
            pltpu.VMEM((S, D), bf16),
            pltpu.VMEM((D, D), bf16),
            pltpu.VMEM((D, F), bf16),
            pltpu.VMEM((F, D), bf16),
            pltpu.VMEM((S // 128, D2, 128), u32),
            pltpu.VMEM((8, S // 2, 128), u32),
            pltpu.VMEM((S // 128, D2, 128), u32),
            pltpu.SemaphoreType.DMA((len(X_SPLIT) - 1,)),
            pltpu.SemaphoreType.DMA((4,)),
            pltpu.SemaphoreType.DMA((5,)),
            pltpu.SemaphoreType.DMA((2,)),
        ],
        compiler_params=pltpu.CompilerParams(vmem_limit_bytes=120 << 20),
    )(A_x, A_wqkv, A_wo, B_w1, B_b1, B_w2, B_b2)
```

```python
import math

import jax
import jax.numpy as jnp
from jax import lax
from jax.experimental import pallas as pl
from jax.experimental.pallas import tpu as pltpu

f32, bf16, u32 = jnp.float32, jnp.bfloat16, jnp.uint32

S, D, H, DH, F = 2048, 1024, 32, 32, 3584
D2, D4, F4 = D // 2, D // 4, F // 4
QB = 256
NQB = S // QB
KC = 128
NC = S // KC
NU = NQB * H
UNROLL = 16
NIT = NU // UNROLL
SKEW = 4
LAG = 6
EPS = 1e-5
QSCALE = (DH ** -0.5) * math.log2(math.e)
X_SPLIT = (0, 256, 512, 1280, 2048)
QUADS = ((0, 0), (0, 1), (1, 0), (1, 1))


def _layernorm(x):
    xc = x - jnp.mean(x, axis=-1, keepdims=True)
    v = jnp.mean(xc * xc, axis=-1, keepdims=True)
    return xc * lax.rsqrt(v + EPS)


def _layernorm_twice(x):
    xc = x - jnp.mean(x, axis=-1, keepdims=True)
    v = jnp.mean(xc * xc, axis=-1, keepdims=True)
    r = lax.rsqrt(v + EPS)
    return xc * (r * lax.rsqrt(v * r * r + EPS))


def _gelu(u):
    c = math.sqrt(2.0 / math.pi)
    z = u * (c + (c * 0.044715) * (u * u))
    hu = 0.5 * u
    return hu + hu * jnp.tanh(z)


def _dot(a, b):
    return jnp.dot(a, b, preferred_element_type=f32)


def _pack(a):
    return pltpu.bitcast(a.astype(bf16), u32)


def _unpack(w):
    return pltpu.bitcast(w, bf16)


def _lhs(ref, p):
    return jnp.concatenate([_unpack(ref[p, t]) for t in range(ref.shape[1])], axis=1)


def _after(x, t):
    t = jnp.tile(t, (x.shape[0] // t.shape[0], x.shape[1] // t.shape[1]))
    return jnp.maximum(x, jnp.minimum(x, t))


def _lhs_factors(a11, a12, a21, a22):
    return [a11 + a22, a21 + a22, a11, a22, a11 + a12, a21 - a11, a12 - a22]


def _rhs_factors(b11, b12, b21, b22):
    return [b11 + b22, b11, b12 - b22, b21 - b11, b22, b11 + b12, b21 + b22]


_RHS_TERMS = ((0, 3, 1), (0, None, 0), (1, 3, -1), (2, 0, -1), (3, None, 0), (0, 1, 1), (2, 3, 1))


def _combine(prod, first=()):
    done = {p: prod(p) for p in first}

    def m(p):
        return done[p] if p in done else prod(p)

    m0 = m(0)
    c11 = m0 + m(6)
    m3 = m(3)
    c11 = c11 + m3
    m4 = m(4)
    c11 = c11 - m4
    m2 = m(2)
    c12 = m2 + m4
    c22 = m0 + m2
    m1 = m(1)
    c21 = m1 + m3
    c22 = (c22 - m1) + m(5)
    return c11, c12, c21, c22


def _lhs_factors2(a):
    outer = [_lhs_factors(a[r][c], a[r][2 + c], a[2 + r][c], a[2 + r][2 + c]) for r, c in QUADS]
    return [v for p in range(7) for v in _lhs_factors(*(outer[q][p] for q in range(4)))]


class _Quad:
    def __init__(self, v):
        self.v = v

    def __add__(self, o):
        return _Quad([a + b for a, b in zip(self.v, o.v)])

    def __sub__(self, o):
        return _Quad([a - b for a, b in zip(self.v, o.v)])


def _inner(prod, p):
    return _Quad(_combine(lambda q: prod(7 * p + q)))


def _combine2(outer):
    out = _combine(outer)
    c = [[None] * 4 for _ in range(4)]
    for po, (ro, co) in enumerate(QUADS):
        for q, (r, cc) in enumerate(QUADS):
            c[2 * ro + r][2 * co + cc] = out[po].v[q]
    return c


def _projections(x_hbm, wqkv_hbm, late_copies, x_s, qT_s, k_s, vT_s, sem_x, sem_k, sem_w,
                 wk_s, wq_s, wv_s, wkb_s, wqb_s, wvb_s, y_s):
    copies = {}
    for i in range(len(X_SPLIT) - 1):
        rows = pl.ds(X_SPLIT[i], X_SPLIT[i + 1] - X_SPLIT[i])
        copies[f"x{i}"] = pltpu.make_async_copy(x_hbm.at[0, rows, :], x_s.at[rows, :], sem_x.at[i])
    for j in range(4):
        copies[f"k{j}"] = pltpu.make_async_copy(
            wqkv_hbm.at[:, pl.ds(D + j * 256, 256)], wk_s.at[j], sem_k.at[j])
    copies["q"] = pltpu.make_async_copy(wqkv_hbm.at[:, pl.ds(0, D)], wq_s, sem_w.at[0])
    copies["v"] = pltpu.make_async_copy(wqkv_hbm.at[:, pl.ds(2 * D, D)], wv_s, sem_w.at[1])

    start_after = {"x0": ("k2",), "k0": ("k3",), "k1": ("x1",), "k2": ("x2",), "x1": ("q", "v"), "x2": ("x3",)}

    def wait(tag):
        copies[tag].wait()
        for t in start_after.get(tag, ()):
            copies[t].start()

    for t in ("x0", "k0", "k1"):
        copies[t].start()

    def ln_piece(i, p, dep=None):
        r = p * 8
        x0 = x_s[i * QB + r:i * QB + r + 8, :].astype(f32)
        x1 = x_s[i * QB + 128 + r:i * QB + 128 + r + 8, :].astype(f32)
        if dep is not None:
            x0 = jnp.concatenate([_after(x0[:, :128], dep), x0[:, 128:]], axis=1)
            x1 = jnp.concatenate([_after(x1[:, :128], dep), x1[:, 128:]], axis=1)
        y0, y1 = _layernorm(x0), _layernorm(x1)
        for n, a in enumerate(_lhs_factors(y0[:, :D2], y0[:, D2:], y1[:, :D2], y1[:, D2:])):
            y_s[n, i * 128 + r:i * 128 + r + 8, :] = a.astype(bf16)

    def weight_sums(src, dst, j, r, dep=None):
        top, bot = src[r:r + 16, :].astype(f32), src[D2 + r:D2 + r + 16, :].astype(f32)
        b11, b12, b21, b22 = top[:, :128], top[:, 128:], bot[:, :128], bot[:, 128:]
        if dep is not None:
            b11, b22 = _after(b11, dep), _after(b22, dep)
        for n, b in enumerate(_rhs_factors(b11, b12, b21, b22)):
            if n not in (1, 4):
                dst[j, n, r:r + 16, :] = b.astype(bf16)

    last = [None]

    def products(src, dst, j, rows, before=None):
        def prod(p):
            if before is not None:
                before()
            if p == 1:
                b = src[:D2, :128]
            elif p == 4:
                b = src[D2:, 128:]
            else:
                b = dst[j, p]
            last[0] = _dot(y_s[p, rows, :], b)
            return last[0]
        return prod

    def sum_jobs(w, wb):
        return [(w.at[:, pl.ds(j * 256, 256)], wb, j, r) for j in range(4) for r in range(0, D2, 16)]

    wait("x0")
    for p in range(16):
        ln_piece(0, p)
    q_jobs = sum_jobs(wq_s, wqb_s)
    for i in range(NQB):
        count = [0]
        ln_from = {0: 22, 1: 15, 4: 15}.get(i, 0)

        def side_work():
            d = count[0]
            count[0] += 1
            if i + 1 < NQB and d >= ln_from:
                n = 26 - ln_from
                for p in range((d - ln_from) * 16 // n, min(16, (d - ln_from + 1) * 16 // n)):
                    ln_piece(i + 1, p, last[0][(p % 4) * 32:(p % 4) * 32 + 8])
            n0 = (i - 4) * 28 + d - 15
            if n0 >= 0:
                for p in range(n0 * len(q_jobs) // 96, min(len(q_jobs), (n0 + 1) * len(q_jobs) // 96)):
                    weight_sums(*q_jobs[p], last[0][32 + 64 * (p % 2):32 + 64 * (p % 2) + 8])

        for j in range(4):
            if i == 0:
                wait(f"k{j}")
                if j == 3:
                    wait("x1")
                for r in range(0, D2, 16):
                    weight_sums(wk_s.at[j], wkb_s, j, r)
            if i == 1 and j == 2:
                wait("x2")
            if i == 4 and j == 2:
                wait("x3")
                wait("q")
                wait("v")
            c = _combine(products(wk_s.at[j], wkb_s, j, slice(i * 128, (i + 1) * 128), side_work),
                         first=(1, 4) if i == 0 else ())
            for (t, g), val in zip(QUADS, c):
                k_s[2 * j + g, i * 128 + t * 64:i * 128 + (t + 1) * 64, :] = _pack(val)

    for copy in late_copies:
        copy.start()
    for w, wb, dst, scale, jobs in ((wq_s, wqb_s, qT_s, QSCALE, sum_jobs(wv_s, wvb_s)),
                                    (wv_s, wvb_s, vT_s, None, [])):
        def next_job():
            if jobs:
                weight_sums(*jobs.pop(0), last[0][32:40])

        for i in range(NQB):
            for j in range(4):
                c = _combine(products(w.at[:, pl.ds(j * 256, 256)], wb, j, slice(i * 128, (i + 1) * 128), next_job))
                for (t, g), val in zip(QUADS, c):
                    if scale is not None:
                        val = val * scale
                    dst[2 * i + t, (2 * j + g) * 64:(2 * j + g + 1) * 64, :] = pltpu.bitcast(
                        val.astype(bf16).T, u32)


def _attention(late_copies, wo_s, w1_s, w2_s, qT_s, k_s, vT_s, wob_s, w1b_s, w2b_s, s_a, s_b, oT_s):
    scores = (s_a, s_b)

    def qk_chunk(u, j, c, s_s, m):
        u = jnp.minimum(u, NU - 1)
        qb, h = u // H, u % H
        ws = []
        for t in range(2):
            parts = [jnp.zeros((16, 128), u32)] * 4
            parts[j] = qT_s[qb * 2 + t, pl.ds(pl.multiple_of(h * 16, 16), 16), :]
            ws.append(_unpack(jnp.concatenate(parts, axis=0)))
        keys = _unpack(k_s[h // 4, c * KC // 2:(c + 1) * KC // 2, :])
        s = _dot(keys, jnp.concatenate(ws, axis=1))
        s_s[c * KC:(c + 1) * KC, :] = s
        for r in range(0, KC, 8):
            m = s[r:r + 8] if m is None else jnp.maximum(m, s[r:r + 8])
        return m

    def row_max(m):
        return jnp.broadcast_to(jnp.max(m, axis=0, keepdims=True), (8, QB))

    def pv_chunk(u, c, s_s, mx, l, acc):
        h = u % H
        ps = []
        for r in range(c * KC, (c + 1) * KC, 16):
            p0 = jnp.exp2(s_s[r:r + 8, :] - mx)
            p1 = jnp.exp2(s_s[r + 8:r + 16, :] - mx)
            l = p0 + p1 if l is None else l + (p0 + p1)
            ps += [p0, p1]
        p = jnp.concatenate(ps, axis=0).astype(bf16)
        a = _dot(_unpack(vT_s[c, pl.ds(pl.multiple_of(h * 16, 16), 16), :]), p)
        return l, (a if acc is None else acc + a)

    def weight_jobs(it):
        jobs = []

        def two_level(src, dst, kq, nq, r0, n, p):
            outer = []

            def blk(r, c):
                return src[pl.ds(r * kq + r0, 16), c * nq + n * 128:c * nq + (n + 1) * 128].astype(f32)

            def emit(qs, dep):
                o = list(outer)
                if dep is not None:
                    o[0], o[3] = _after(o[0], dep), _after(o[3], dep)
                vals = _rhs_factors(*o)
                for q in qs:
                    dst[7 * p + q, n, pl.ds(pl.multiple_of(r0 // 2, 8), 8), :] = _pack(vals[q])

            def begin(dep):
                qa, qb, sign = _RHS_TERMS[p]
                for r, c in QUADS:
                    v = blk(2 * QUADS[qa][0] + r, 2 * QUADS[qa][1] + c)
                    if r == c:
                        v = _after(v, dep)
                    if sign:
                        v2 = blk(2 * QUADS[qb][0] + r, 2 * QUADS[qb][1] + c)
                        v = v + v2 if sign > 0 else v - v2
                    outer.append(v)
                emit(range(3), None)

            jobs.append(begin)
            jobs.append(lambda dep: emit(range(3, 7), dep))

        def one_level(r0, j):
            def run(dep):
                top = _after(wo_s[pl.ds(r0, 16), j * 256:(j + 1) * 256].astype(f32), dep)
                bot = wo_s[pl.ds(D2 + r0, 16), j * 256:(j + 1) * 256].astype(f32)
                for n, b in enumerate(_rhs_factors(top[:, :128], top[:, 128:], bot[:, :128], bot[:, 128:])):
                    wob_s[j, n, pl.ds(pl.multiple_of(r0 // 2, 8), 8), :] = _pack(b)
            jobs.append(run)

        def row_groups(total):
            groups = total // 16
            per_step = -(-groups // NIT)
            starts = [it * per_step + a for a in range(per_step)]
            if per_step * NIT > groups:
                starts = [jnp.minimum(g, groups - 1) for g in starts]
            return [pl.multiple_of(g * 16, 16) for g in starts]

        for src, dst, kq, nq in ((w1_s, w1b_s, D4, F4), (w2_s, w2b_s, F4, D4)):
            for r0 in row_groups(kq):
                for n in range(nq // 128):
                    for p in range(7):
                        two_level(src, dst, kq, nq, r0, n, p)
        for r0 in row_groups(D2):
            for j in range(4):
                one_level(r0, j)
        return jobs

    def unit(it, j, mx, m, hist, jobs):
        u = UNROLL * it + j
        l = acc = mx_next = None
        for c in range(NC):
            cq = c + SKEW
            if cq < NC:
                m = qk_chunk(u + 1, (j + 1) % 4, cq, scores[(j + 1) % 2], m)
                if cq == NC - 1:
                    mx_next, m = row_max(m), None
            else:
                m = qk_chunk(u + 2, (j + 2) % 4, cq - NC, scores[j % 2], m)
            hist.append(m if m is not None else mx_next)
            n0, n1 = j * NC + c, UNROLL * NC
            for p in range(n0 * len(jobs) // n1, (n0 + 1) * len(jobs) // n1):
                jobs[p](hist[-1][:, :128])
            mxc = _after(mx, hist[-LAG]) if len(hist) >= LAG else mx
            l, acc = pv_chunk(u, c, scores[j % 2], mxc, l, acc)
        o = acc * (1.0 / jnp.sum(l, axis=0, keepdims=True))
        for t in range(2):
            oT_s[(u // H) * 2 + t, pl.ds(pl.multiple_of((u % H) * DH, DH), DH), :] = o[:, t * 128:(t + 1) * 128]
        return mx_next, m

    m = None
    for c in range(NC):
        m = qk_chunk(0, 0, c, s_a, m)
    mx, m = row_max(m), None
    for c in range(SKEW):
        m = qk_chunk(1, 1, c, s_b, m)
    for copy in late_copies:
        copy.wait()

    def step(it, carry):
        mx, m = carry
        hist = []
        jobs = weight_jobs(it)
        for j in range(UNROLL):
            mx, m = unit(it, j, mx, m, hist, jobs)
        return mx, m

    lax.fori_loop(0, NIT, step, (mx, m))


def _mix(b1_ref, b2_ref, out_hbm, x_s, sem_o, wob_s, w1b_s, w2b_s, oT_s, oa_s, h_s, y0_s, ya_s, ua_s, out_s):
    def out_copy(qb, slot):
        return pltpu.make_async_copy(
            out_s.at[slot], out_hbm.at[0, pl.ds(pl.multiple_of(qb * QB, QB), QB), :], sem_o.at[slot])

    def o_factors(qb, t, g, dep=None):
        lo = oT_s[2 * qb + t, g * 128:(g + 1) * 128, :]
        hi = oT_s[2 * qb + t, D2 + g * 128:D2 + (g + 1) * 128, :]
        if dep is not None:
            lo, hi = _after(lo, dep), _after(hi, dep)
        lo, hi = lo.T, hi.T
        for n, a in enumerate(_lhs_factors(lo[:64], hi[:64], lo[64:], hi[64:])):
            oa_s[7 * t + n, g] = _pack(a)

    def blocks(ys, kt):
        return [[y[:, cq * D4 + kt * 128:cq * D4 + (kt + 1) * 128] for cq in range(4)] for y in ys]

    def step(qb, carry):
        slot = qb % 2

        @pl.when(qb >= 2)
        def _():
            out_copy(qb - 2, slot).wait()

        b1 = b1_ref[...].astype(f32).reshape(1, F)
        b2 = b2_ref[...].astype(f32).reshape(1, D)
        r0 = pl.multiple_of(qb * QB, QB)

        for t in range(2):
            for j in range(4):
                c = _combine(lambda p: _dot(_lhs(oa_s, 7 * t + p), _unpack(wob_s[j, p])))
                for (r, g), val in zip(QUADS, c):
                    cs = slice((2 * j + g) * 128, (2 * j + g + 1) * 128)
                    ro = t * 128 + r * 64
                    h_s[ro:ro + 64, cs] = x_s[pl.ds(r0 + ro, 64), cs].astype(f32) + val
            for r in range(0, 64, 16):
                ys = [_layernorm_twice(h_s[t * 128 + q * 64 + r:t * 128 + q * 64 + r + 16, :]) for q in range(2)]
                if t == 0:
                    for q in range(2):
                        y0_s[q * 64 + r:q * 64 + r + 16, :] = ys[q]
                    for kt in range(2):
                        a = blocks(ys, kt)
                        top = [(a[q][cc], a[q][cc] + a[q][2 + cc]) for q, cc in QUADS]
                        for p, sel in ((2, 0), (4, 1)):
                            for n, v in enumerate(_lhs_factors(*(o[sel] for o in top))):
                                ya_s[7 * p + n, kt, r // 2:r // 2 + 8, :] = _pack(v)
                else:
                    ys = [y0_s[q * 64 + r:q * 64 + r + 16, :] for q in range(2)] + ys
                    for kt in range(2):
                        for n, v in enumerate(_lhs_factors2(blocks(ys, kt))):
                            if n // 7 not in (2, 4):
                                ya_s[n, kt, r // 2:r // 2 + 8, :] = _pack(v)

        def up(n, p):
            return _inner(lambda q: _dot(_lhs(ya_s, q), _unpack(w1b_s[q, n])), p)

        ahead = {(n, p): up(n, p) for n in range(2) for p in (2, 4)}
        for n in range(F4 // 128):
            c = _combine2(lambda p: ahead[n, p] if (n, p) in ahead else up(n, p))
            for r in range(0, 64, 16):
                u = [[_gelu(c[t][cq][r:r + 16] + b1[:, cq * F4 + n * 128:cq * F4 + (n + 1) * 128])
                      for cq in range(4)] for t in range(4)]
                for p, a in enumerate(_lhs_factors2(u)):
                    ua_s[p, n, r // 2:r // 2 + 8, :] = _pack(a)

        nxt = jnp.minimum(qb + 1, NQB - 1)
        for n in range(D4 // 128):
            count = [0]

            def prod(p):
                val = _dot(_lhs(ua_s, p), _unpack(w2b_s[p, n]))
                if count[0] % 12 == 8:
                    o_factors(nxt, n, count[0] // 12, val[:8])
                count[0] += 1
                return val

            c = _combine2(lambda p: _inner(prod, p))
            for t in range(4):
                for cq in range(4):
                    rs, cs = slice(t * 64, (t + 1) * 64), slice(cq * D4 + n * 128, cq * D4 + (n + 1) * 128)
                    out_s[slot, rs, cs] = (h_s[rs, cs] + (c[t][cq] + b2[:, cs])).astype(bf16)
        out_copy(qb, slot).start()
        return carry

    for t in range(2):
        for g in range(4):
            o_factors(0, t, g)
    lax.fori_loop(0, NQB, step, 0)
    out_copy(NQB - 2, 0).wait()
    out_copy(NQB - 1, 1).wait()


def _kernel(x_hbm, wqkv_hbm, wo_hbm, w1_hbm, b1_ref, w2_hbm, b2_ref, out_hbm,
            x_s, wo_s, w1_s, w2_s, qT_s, k_s, vT_s, sem_x, sem_k, sem_w, sem_o):
    late_copies = (pltpu.make_async_copy(w1_hbm, w1_s, sem_w.at[2]),
                   pltpu.make_async_copy(w2_hbm, w2_s, sem_w.at[3]),
                   pltpu.make_async_copy(wo_hbm, wo_s, sem_w.at[4]))

    def first(*bufs):
        _projections(x_hbm, wqkv_hbm, late_copies, x_s, qT_s, k_s, vT_s, sem_x, sem_k, sem_w, *bufs)

    pl.run_scoped(
        first,
        pltpu.VMEM((4, D, 256), bf16),
        pltpu.VMEM((D, D), bf16),
        pltpu.VMEM((D, D), bf16),
        pltpu.VMEM((4, 7, D2, 128), bf16),
        pltpu.VMEM((4, 7, D2, 128), bf16),
        pltpu.VMEM((4, 7, D2, 128), bf16),
        pltpu.VMEM((7, S // 2, D2), bf16))

    def second(wob_s, w1b_s, w2b_s, s_a, s_b, oT_s, *bufs):
        _attention(late_copies, wo_s, w1_s, w2_s, qT_s, k_s, vT_s, wob_s, w1b_s, w2b_s, s_a, s_b, oT_s)
        _mix(b1_ref, b2_ref, out_hbm, x_s, sem_o, wob_s, w1b_s, w2b_s, oT_s, *bufs)

    pl.run_scoped(
        second,
        pltpu.VMEM((4, 7, D2 // 2, 128), u32),
        pltpu.VMEM((49, F4 // 128, D4 // 2, 128), u32),
        pltpu.VMEM((49, D4 // 128, F4 // 2, 128), u32),
        pltpu.VMEM((S, QB), f32),
        pltpu.VMEM((S, QB), f32),
        pltpu.VMEM((S // 128, D, 128), f32),
        pltpu.VMEM((14, 4, 32, 128), u32),
        pltpu.VMEM((QB, D), f32),
        pltpu.VMEM((128, D), f32),
        pltpu.VMEM((49, D4 // 128, 32, 128), u32),
        pltpu.VMEM((49, F4 // 128, 32, 128), u32),
        pltpu.VMEM((2, QB, D), bf16))


@jax.jit
def pallas_sequential_preLN__softmax_full_mha__mixer_channel_mlp__prompt_kernel(
    A_x: jax.Array,
    A_wqkv: jax.Array,
    A_wo: jax.Array,
    B_x: jax.Array,
    B_w1: jax.Array,
    B_b1: jax.Array,
    B_w2: jax.Array,
    B_b2: jax.Array,
):
    del B_x
    hbm = pl.BlockSpec(memory_space=pl.ANY)
    vmem = pl.BlockSpec(memory_space=pltpu.VMEM)
    return pl.pallas_call(
        _kernel,
        out_shape=jax.ShapeDtypeStruct((1, S, D), bf16),
        in_specs=[hbm, hbm, hbm, hbm, vmem, hbm, vmem],
        out_specs=hbm,
        scratch_shapes=[
            pltpu.VMEM((S, D), bf16),
            pltpu.VMEM((D, D), bf16),
            pltpu.VMEM((D, F), bf16),
            pltpu.VMEM((F, D), bf16),
            pltpu.VMEM((S // 128, D2, 128), u32),
            pltpu.VMEM((8, S // 2, 128), u32),
            pltpu.VMEM((S // 128, D2, 128), u32),
            pltpu.SemaphoreType.DMA((len(X_SPLIT) - 1,)),
            pltpu.SemaphoreType.DMA((4,)),
            pltpu.SemaphoreType.DMA((5,)),
            pltpu.SemaphoreType.DMA((2,)),
        ],
        compiler_params=pltpu.CompilerParams(vmem_limit_bytes=120 << 20),
    )(A_x, A_wqkv, A_wo, B_w1, B_b1, B_w2, B_b2)
```
